```python
import jax
import jax.numpy as jnp

def _softmax(x, axis=-1):
    return jax.nn.softmax(x, axis=axis)

def _gelu(x):
    return jax.nn.gelu(x, approximate=True)

def _silu(x):
    return jax.nn.silu(x)

def _sigmoid(x):
    return jax.nn.sigmoid(x)

def _layernorm(x, axis=-1, eps=1e-05):
    m = jnp.mean(x, axis=axis, keepdims=True)
    v = jnp.var(x, axis=axis, keepdims=True)
    return (x - m) / jnp.sqrt(v + eps)

def _scatter_add(tgt, idx, src, axis=0):
    return tgt.at[idx].add(src)

def _segment_sum(src, seg, n):
    return jax.ops.segment_sum(src, seg, n)

class _Rng:

    def __init__(self, key):
        self._k = key

    def _next(self):
        self._k, sub = jax.random.split(self._k)
        return sub

    def normal(self, shape):
        return jax.random.normal(self._next(), shape, dtype=jnp.bfloat16)

    def randint(self, lo, hi, shape):
        return jax.random.randint(self._next(), shape, lo, hi, dtype=jnp.int32)

    def uniform(self, shape, lo=0.0, hi=1.0):
        return jax.random.uniform(self._next(), shape, jnp.bfloat16, lo, hi)

    def permutation(self, n):
        return jax.random.permutation(self._next(), n)
kernel_name = 'adaLN_cond__memory_aug_recurrent_mem_tr__mixer_s_mlp__prompt'

def setup_inputs():
    _rng = _Rng(jax.random.key(int.from_bytes(__import__("os").urandom(4), "little")))
    _w = lambda a: (lambda t: t.astype(jnp.bfloat16) if jnp.issubdtype(t.dtype, jnp.floating) else t)(jnp.asarray(a))

    def _A_setup():
        B, S, Dm = (1, 2048, 1024)
        H, Dh = (32, 128)
        M, seg = (8, 32)
        seg = min(seg, S)
        S = S // seg * seg
        return {'x': _w((lambda *s: _rng.normal(s) * 0.05)(B, S, Dm)), 'mem0': _w((lambda *s: _rng.normal(s) * 0.05)(B, M, Dm)), 'Wq': _w((lambda *s: _rng.normal(s) * 0.05)(Dm, H, Dh) * Dm ** (-0.5)), 'Wk': _w((lambda *s: _rng.normal(s) * 0.05)(Dm, H, Dh) * Dm ** (-0.5)), 'Wv': _w((lambda *s: _rng.normal(s) * 0.05)(Dm, H, Dh) * Dm ** (-0.5)), 'Wo': _w((lambda *s: _rng.normal(s) * 0.05)(H, Dh, Dm) * (H * Dh) ** (-0.5)), 'seg_len': seg}
    _A_in = _A_setup()

    def _B_setup():
        B, S, D, F = (1, 2048, 1024, 3584)
        return {'x': _w((lambda *s: _rng.normal(s) * 0.05)(B, S, D)), 'w1': _w((lambda *s: _rng.normal(s) * 0.05)(D, D) * D ** (-0.5)), 'w2': _w((lambda *s: _rng.normal(s) * 0.05)(D, D) * D ** (-0.5)), 'w3': _w((lambda *s: _rng.normal(s) * 0.05)(D, F) * D ** (-0.5)), 'w4': _w((lambda *s: _rng.normal(s) * 0.05)(F, D) * F ** (-0.5))}
    _B_in = _B_setup()
    return {'A_x': _A_in['x'], 'A_mem0': _A_in['mem0'], 'A_Wq': _A_in['Wq'], 'A_Wk': _A_in['Wk'], 'A_Wv': _A_in['Wv'], 'A_Wo': _A_in['Wo'], 'A_seg_len': _A_in['seg_len'], 'B_x': _B_in['x'], 'B_w1': _B_in['w1'], 'B_w2': _B_in['w2'], 'B_w3': _B_in['w3'], 'B_w4': _B_in['w4'], 'c': _w((lambda *s: _rng.normal(s) * 0.05)(1, 1024)), 'w_mod': _w((lambda *s: _rng.normal(s) * 0.05)(1024, 6 * 1024) * 1024 ** (-0.5))}

def reference(A_x, A_mem0, A_Wq, A_Wk, A_Wv, A_Wo, A_seg_len, B_x, B_w1, B_w2, B_w3, B_w4, c, w_mod):

    def _A_ref(x, mem0, Wq, Wk, Wv, Wo, seg_len):
        B, S, Dm = x.shape
        H, Dh = (Wq.shape[1], Wq.shape[2])
        M = mem0.shape[1]
        scale = Dh ** (-0.5)
        n_seg = S // seg_len
        L = M + seg_len
        idx = jnp.arange(L)
        mask = (idx[:, None] < M) | (idx[:, None] >= idx[None, :])
        mem = mem0
        outs = []
        for s in range(n_seg):
            xs = x[:, s * seg_len:(s + 1) * seg_len, :].copy()
            h = jnp.concatenate([mem, xs], axis=1)
            q = jnp.einsum('btd,dhe->bhte', h, Wq)
            k = jnp.einsum('btd,dhe->bhte', h, Wk)
            v = jnp.einsum('btd,dhe->bhte', h, Wv)
            scores = jnp.einsum('bhqe,bhke->bhqk', q, k) * scale
            scores = jnp.where(mask[None, None], scores, -1000000000.0)
            p = _softmax(scores, axis=-1)
            o = jnp.einsum('bhqk,bhke->bhqe', p, v)
            o = jnp.einsum('bhte,hed->btd', o, Wo)
            mem = o[:, :M, :].copy()
            outs.append(o[:, M:, :])
        return jnp.concatenate(outs, axis=1)

    def _B_ref(x, w1, w2, w3, w4):
        B, S, D = x.shape
        h = _gelu(_layernorm(x, axis=-1) @ w1)
        c = D // 4
        g0 = jnp.pad(h[:, :, 0 * c:1 * c], ((0, 0), (1, 0), (0, 0)))[:, :S, :]
        g1 = jnp.pad(h[:, :, 1 * c:2 * c], ((0, 0), (0, 1), (0, 0)))[:, 1:, :]
        g2 = jnp.pad(h[:, :, 2 * c:3 * c], ((0, 0), (2, 0), (0, 0)))[:, :S, :]
        g3 = jnp.pad(h[:, :, 3 * c:], ((0, 0), (0, 2), (0, 0)))[:, 2:, :]
        hs = jnp.concatenate([g0, g1, g2, g3], axis=-1) @ w2
        x1 = x + hs
        h2 = _gelu(_layernorm(x1, axis=-1) @ w3) @ w4
        return x1 + h2
    x = A_x
    mod = (_silu(c) @ w_mod).reshape(c.shape[0], 6, 1, -1)
    sa, ca, ga, sb, cb, gb = (mod[:, 0].copy(), mod[:, 1].copy(), mod[:, 2].copy(), mod[:, 3].copy(), mod[:, 4].copy(), mod[:, 5].copy())
    h = _layernorm(x, axis=-1) * (1 + ca) + sa
    x = x + ga * _A_ref(h, A_mem0, A_Wq, A_Wk, A_Wv, A_Wo, A_seg_len)
    h = _layernorm(x, axis=-1) * (1 + cb) + sb
    x = x + gb * _B_ref(h, B_w1, B_w2, B_w3, B_w4)
    return x
```

```python
import functools

import jax
import jax.numpy as jnp
from jax import lax
import jax.experimental.pallas as pl
import jax.experimental.pallas.tpu as pltpu

F32 = jnp.float32
BF16 = jnp.bfloat16
LANES = 128
HEAD_TILE = 8
EPS = 1e-5

_NN = (((1,), (0,)), ((), ()))
_NT = (((1,), (1,)), ((), ()))


def _mm(a, b, dims=_NN):
    return lax.dot_general(a, b, dims, preferred_element_type=F32)


def _layernorm(x):
    m = jnp.mean(x, axis=-1, keepdims=True)
    d = x - m
    v = jnp.mean(d * d, axis=-1, keepdims=True)
    return d * lax.rsqrt(v + EPS)


def _gelu(x):
    k = 0.7978845608028654
    return (0.5 * x) * (1.0 + jnp.tanh(k * (x + 0.044715 * (x * x * x))))


def _kernel(
    x_hbm, mem0_ref, wq_hbm, wk_hbm, wv_hbm, wo_hbm,
    w1_hbm, w2_hbm, w3_hbm, w4_hbm, c_ref, wmod_hbm,
    out_hbm,
    x_s, hbuf, wqkv_s, wo_s, stage, wmod_s, mod_s,
    w1_s, w2_s, w3_s, w4_s, u_s, o_s, out_s,
    sem_x, sem_stage, sem_wo, sem_mod, sem_b, sem_out,
    *, S, D, H, Dh, M, seg, F, RB,
):
    n_seg = S // seg
    L = M + seg
    n_col = D // LANES
    scale = Dh ** (-0.5)
    PAD = 8

    def mod_copy(j):
        return pltpu.make_async_copy(
            wmod_hbm.at[:, pl.ds(j * 2 * D, 2 * D)], wmod_s.at[j], sem_mod.at[j])

    x_copy = pltpu.make_async_copy(x_hbm, x_s, sem_x)

    w_chunks = [(m, t) for t in range(H // HEAD_TILE) for m in range(3)]
    w_hbm = (wq_hbm, wk_hbm, wv_hbm)

    def stage_copy(i):
        m, t = w_chunks[i]
        return pltpu.make_async_copy(
            w_hbm[m].at[:, pl.ds(t * HEAD_TILE, HEAD_TILE), :],
            stage.at[i % 2], sem_stage.at[i % 2])

    def wo_copy(j):
        return pltpu.make_async_copy(
            wo_hbm.at[:, pl.ds(j * LANES, LANES)], wo_s.at[j], sem_wo.at[j])

    b_copies = [
        pltpu.make_async_copy(src, dst, sem_b.at[i])
        for i, (src, dst) in enumerate(
            ((w1_hbm, w1_s), (w2_hbm, w2_s), (w3_hbm, w3_s), (w4_hbm, w4_s)))
    ]

    mod_copy(0).start()
    x_copy.start()
    stage_copy(0).start()
    stage_copy(1).start()

    cv = c_ref[...].astype(F32)
    sc = jnp.broadcast_to(cv * (1.0 / (1.0 + jnp.exp(-cv))), (8, D))

    def make_mod(j):
        mod_copy(j).wait()
        r = _mm(sc, wmod_s[j])
        mod_s[2 * j] = r[:, :D]
        mod_s[2 * j + 1] = r[:, D:]

    make_mod(0)
    x_copy.wait()

    def ln_body(s, carry):
        xs = x_s[pl.ds(pl.multiple_of(s * seg, seg), seg), :].astype(F32)
        hbuf[s, M:, :] = _layernorm(xs) * (1.0 + mod_s[1, 0:1, :]) + mod_s[0, 0:1, :]
        return carry

    lax.fori_loop(0, n_seg, ln_body, 0, unroll=4)
    hbuf[0, :M, :] = mem0_ref[...].astype(F32)

    for i, (m, t) in enumerate(w_chunks):
        stage_copy(i).wait()

        def retile(r, carry, i=i, m=m, t=t):
            rows = pl.ds(pl.multiple_of(r * 64, 64), 64)
            blk = jnp.transpose(stage[i % 2, rows, :, :], (1, 0, 2))
            wqkv_s[m, pl.ds(t * HEAD_TILE, HEAD_TILE), rows, :] = blk
            return carry

        lax.fori_loop(0, D // 64, retile, 0)
        if i + 2 < len(w_chunks):
            stage_copy(i + 2).start()
        elif i + 2 == len(w_chunks):
            for j in range(n_col):
                wo_copy(j).start()

    mod_copy(1).start()
    mod_copy(2).start()
    for cp in b_copies:
        cp.start()
    for j in range(n_col):
        wo_copy(j).wait()

    row = lax.broadcasted_iota(jnp.int32, (L, L), 0)
    col = lax.broadcasted_iota(jnp.int32, (L, L), 1)
    mask = (row < M) | (row >= col)
    half = (H // 2) * Dh

    def step(s, carry):
        for h in range(H):
            hc = hbuf[s]
            q = _mm(hc, wqkv_s[0, h])
            k = _mm(hc, wqkv_s[1, h]).astype(BF16)
            v = _mm(hc, wqkv_s[2, h]).astype(BF16)
            sc_ = jnp.where(mask, _mm(q, k, _NT) * scale, -1000000000.0)
            e = jnp.exp(sc_ - jnp.max(sc_, axis=-1, keepdims=True))
            inv = 1.0 / jnp.sum(e, axis=-1, keepdims=True)
            o_s[:, h * Dh:(h + 1) * Dh] = _mm(e, v) * inv
        first = [_mm(o_s[:, :half], wo_s[j, :half, :]) for j in range(n_col)]
        nxt = jnp.minimum(s + 1, n_seg)
        for j in range(n_col):
            r = first[j] + _mm(o_s[:, half:], wo_s[j, half:, :])
            cols = slice(j * LANES, (j + 1) * LANES)
            hbuf[nxt, :M, cols] = r[:M]
            hbuf[s, M:, cols] = r[M:]
        return carry

    lax.fori_loop(0, n_seg, step, 0)

    make_mod(1)
    make_mod(2)
    for cp in b_copies:
        cp.wait()

    spb = RB // seg
    n_chunk = S // RB

    def resid(i):
        rows = pl.ds(pl.multiple_of(i * RB, RB), RB)
        a = hbuf[pl.ds(i * spb, spb), M:, :].reshape(RB, D)
        xa = x_s[rows, :].astype(F32) + mod_s[2, 0:1, :] * a
        hb = _layernorm(xa) * (1.0 + mod_s[4, 0:1, :]) + mod_s[3, 0:1, :]
        return xa, hb

    u_s[:PAD, :] = jnp.zeros((PAD, D), F32)
    u_s[PAD + S:, :] = jnp.zeros((PAD, D), F32)

    def mix_in(i, carry):
        _, hb = resid(i)
        u = _gelu(_mm(_layernorm(hb).astype(BF16), w1_s[...]))
        u_s[pl.ds(pl.multiple_of(PAD + i * RB, 8), RB), :] = u
        return carry

    lax.fori_loop(0, n_chunk, mix_in, 0)

    def out_copy(i, slot):
        return pltpu.make_async_copy(
            out_s.at[slot], out_hbm.at[pl.ds(pl.multiple_of(i * RB, RB), RB), :],
            sem_out.at[slot])

    cq = D // 4

    def mlp(i, carry):
        slot = i % 2
        xa, hb = resid(i)
        win = pl.ds(pl.multiple_of(i * RB, 8), RB + 2 * PAD)
        parts = []
        for g, off in enumerate((-1, 1, -2, 2)):
            ug = u_s[win, g * cq:(g + 1) * cq]
            parts.append(ug[PAD + off:PAD + off + RB].astype(BF16))
        x1 = hb + _mm(jnp.concatenate(parts, axis=1), w2_s[...])
        t = _gelu(_mm(_layernorm(x1).astype(BF16), w3_s[...]))
        y = x1 + _mm(t.astype(BF16), w4_s[...])
        res = (xa + mod_s[5, 0:1, :] * y).astype(out_s.dtype)

        @pl.when(i >= 2)
        def _():
            out_copy(i - 2, slot).wait()

        out_s[slot] = res
        out_copy(i, slot).start()
        return carry

    lax.fori_loop(0, n_chunk, mlp, 0)
    out_copy(n_chunk - 2, (n_chunk - 2) % 2).wait()
    out_copy(n_chunk - 1, (n_chunk - 1) % 2).wait()


@functools.partial(jax.jit, static_argnames=("A_seg_len",))
def pallas_adaLN_cond__memory_aug_recurrent_mem_tr__mixer_s_mlp__prompt_kernel(
    A_x, A_mem0, A_Wq, A_Wk, A_Wv, A_Wo, A_seg_len,
    B_x, B_w1, B_w2, B_w3, B_w4, c, w_mod,
):
    del B_x
    B, S, D = A_x.shape
    _, H, Dh = A_Wq.shape
    M = A_mem0.shape[1]
    F = B_w3.shape[1]
    seg = int(A_seg_len)
    RB = 256
    assert B == 1 and Dh == LANES and S % RB == 0 and RB % seg == 0
    n_seg = S // seg

    hbm = pl.BlockSpec(memory_space=pl.ANY)
    vmem = pl.BlockSpec(memory_space=pltpu.VMEM)
    dma = pltpu.SemaphoreType.DMA

    out = pl.pallas_call(
        functools.partial(_kernel, S=S, D=D, H=H, Dh=Dh, M=M, seg=seg, F=F, RB=RB),
        out_shape=jax.ShapeDtypeStruct((S, D), A_x.dtype),
        in_specs=[hbm, vmem, hbm, hbm, hbm, hbm, hbm, hbm, hbm, hbm, vmem, hbm],
        out_specs=hbm,
        scratch_shapes=[
            pltpu.VMEM((S, D), A_x.dtype),
            pltpu.VMEM((n_seg + 1, M + seg, D), F32),
            pltpu.VMEM((3, H, D, Dh), BF16),
            pltpu.VMEM((D // LANES, H * Dh, LANES), BF16),
            pltpu.VMEM((2, D, HEAD_TILE, Dh), BF16),
            pltpu.VMEM((3, D, 2 * D), BF16),
            pltpu.VMEM((6, 8, D), F32),
            pltpu.VMEM((D, D), BF16),
            pltpu.VMEM((D, D), BF16),
            pltpu.VMEM((D, F), BF16),
            pltpu.VMEM((F, D), BF16),
            pltpu.VMEM((S + 16, D), F32),
            pltpu.VMEM((M + seg, H * Dh), F32),
            pltpu.VMEM((2, RB, D), A_x.dtype),
            dma(()), dma((2,)), dma((D // LANES,)), dma((3,)), dma((4,)), dma((2,)),
        ],
        compiler_params=pltpu.CompilerParams(vmem_limit_bytes=120 * 1024 * 1024),
    )(
        A_x.reshape(S, D), A_mem0.reshape(M, D), A_Wq, A_Wk, A_Wv,
        A_Wo.reshape(H * Dh, D), B_w1, B_w2, B_w3, B_w4, c, w_mod,
    )
    return out.reshape(B, S, D)
```

```python
import functools

import jax
import jax.numpy as jnp
from jax import lax
import jax.experimental.pallas as pl
import jax.experimental.pallas.tpu as pltpu

F32 = jnp.float32
BF16 = jnp.bfloat16
U32 = jnp.uint32
LANES = 128
HEAD_TILE = 8
EPS = 1e-5

_NN = (((1,), (0,)), ((), ()))
_NT = (((1,), (1,)), ((), ()))


def _mm(a, b, dims=_NN):
    return lax.dot_general(a, b, dims, preferred_element_type=F32)


def _bf(w):
    return pltpu.bitcast(w, BF16)


def _layernorm(x):
    m = jnp.mean(x, axis=-1, keepdims=True)
    d = x - m
    v = jnp.mean(d * d, axis=-1, keepdims=True)
    return d * lax.rsqrt(v + EPS)


def _gelu(x):
    k = 0.7978845608028654
    return (0.5 * x) * (1.0 + jnp.tanh(k * (x + 0.044715 * (x * x * x))))


def _kernel(
    x_hbm, mem0_ref, wq_hbm, wk_hbm, wv_hbm, wo_hbm,
    w1_hbm, w2_hbm, w3_hbm, w4_hbm, c_ref, wmod_hbm,
    out_hbm,
    x_s, hbuf, wqkv_s, wo_s, stage, wmod_s, mod_s,
    w1_s, w2_s, w3_s, w4_s, u_s, o_s, out_s,
    sem_x, sem_stage, sem_wo, sem_mod, sem_b, sem_out,
    *, S, D, H, Dh, M, seg, F, RB,
):
    n_seg = S // seg
    L = M + seg
    n_col = D // LANES
    scale = Dh ** (-0.5)
    PAD = 8

    def mod_copy(j):
        return pltpu.make_async_copy(
            wmod_hbm.at[:, pl.ds(j * 2 * D, 2 * D)], wmod_s.at[j], sem_mod.at[j])

    x_copy = pltpu.make_async_copy(x_hbm, x_s, sem_x)

    w_chunks = [(m, t) for t in range(H // HEAD_TILE) for m in range(3)]
    w_hbm = (wq_hbm, wk_hbm, wv_hbm)

    def stage_copy(i):
        m, t = w_chunks[i]
        return pltpu.make_async_copy(
            w_hbm[m].at[:, pl.ds(t * HEAD_TILE, HEAD_TILE), :],
            stage.at[i % 2], sem_stage.at[i % 2])

    def wo_copy(j):
        return pltpu.make_async_copy(
            wo_hbm.at[:, pl.ds(j * LANES, LANES)], wo_s.at[j], sem_wo.at[j])

    b_copies = [
        pltpu.make_async_copy(src, dst, sem_b.at[i])
        for i, (src, dst) in enumerate(
            ((w1_hbm, w1_s), (w2_hbm, w2_s), (w3_hbm, w3_s), (w4_hbm, w4_s)))
    ]

    mod_copy(0).start()
    x_copy.start()
    stage_copy(0).start()
    stage_copy(1).start()

    cv = c_ref[...].astype(F32)
    sc = jnp.broadcast_to(cv * (1.0 / (1.0 + jnp.exp(-cv))), (8, D))

    def make_mod(j):
        mod_copy(j).wait()
        r = _mm(sc, wmod_s[j])
        mod_s[2 * j] = r[:, :D]
        mod_s[2 * j + 1] = r[:, D:]

    make_mod(0)
    x_copy.wait()

    def ln_body(s, carry):
        xs = x_s[pl.ds(pl.multiple_of(s * seg, seg), seg), :].astype(F32)
        hbuf[s, M:, :] = _layernorm(xs) * (1.0 + mod_s[1, 0:1, :]) + mod_s[0, 0:1, :]
        return carry

    lax.fori_loop(0, n_seg, ln_body, 0, unroll=4)
    hbuf[0, :M, :] = mem0_ref[...].astype(F32)

    for i, (m, t) in enumerate(w_chunks):
        stage_copy(i).wait()

        def retile(r, carry, i=i, m=m, t=t):
            rows = pl.ds(pl.multiple_of(r * 64, 64), 64)
            blk = jnp.transpose(stage[i % 2, rows, :, :], (1, 0, 2))
            half_rows = pl.ds(pl.multiple_of(r * 32, 32), 32)
            for hh in range(HEAD_TILE):
                wqkv_s[m, t * HEAD_TILE + hh, half_rows, :] = pltpu.bitcast(blk[hh], U32)
            return carry

        lax.fori_loop(0, D // 64, retile, 0)
        if i + 2 < len(w_chunks):
            stage_copy(i + 2).start()
        elif i + 2 == len(w_chunks):
            for j in range(n_col):
                wo_copy(j).start()

    mod_copy(1).start()
    mod_copy(2).start()
    for cp in b_copies:
        cp.start()
    for j in range(n_col):
        wo_copy(j).wait()

    row = lax.broadcasted_iota(jnp.int32, (L, L), 0)
    col = lax.broadcasted_iota(jnp.int32, (L, L), 1)
    mask = (row < M) | (row >= col)
    half = (H // 2) * Dh

    def step(s, carry):
        qkv, ev = {}, {}
        for t in range(H + 2):
            if t < H:
                hc = hbuf[s]
                qkv[t] = (_mm(hc, _bf(wqkv_s[0, t])),
                          _mm(hc, _bf(wqkv_s[1, t])).astype(BF16),
                          _mm(hc, _bf(wqkv_s[2, t])).astype(BF16))
            if 0 <= t - 1 < H:
                q, k, v = qkv.pop(t - 1)
                sc_ = jnp.where(mask, _mm(q, k, _NT) * scale, -1000000000.0)
                e = jnp.exp(sc_ - jnp.max(sc_, axis=-1, keepdims=True))
                ev[t - 1] = (e, v)
            if 0 <= t - 2 < H:
                h = t - 2
                e, v = ev.pop(h)
                inv = 1.0 / jnp.sum(e, axis=-1, keepdims=True)
                o_s[:, h * Dh:(h + 1) * Dh] = _mm(e, v) * inv
        first = [_mm(o_s[:, :half], wo_s[j, :half, :]) for j in range(n_col)]
        nxt = jnp.minimum(s + 1, n_seg)
        for j in range(n_col):
            r = first[j] + _mm(o_s[:, half:], wo_s[j, half:, :])
            cols = slice(j * LANES, (j + 1) * LANES)
            hbuf[nxt, :M, cols] = r[:M]
            hbuf[s, M:, cols] = r[M:]
        return carry

    lax.fori_loop(0, n_seg, step, 0)

    make_mod(1)
    make_mod(2)
    for cp in b_copies:
        cp.wait()

    spb = RB // seg
    n_chunk = S // RB

    def resid(i):
        rows = pl.ds(pl.multiple_of(i * RB, RB), RB)
        a = hbuf[pl.ds(i * spb, spb), M:, :].reshape(RB, D)
        xa = x_s[rows, :].astype(F32) + mod_s[2, 0:1, :] * a
        hb = _layernorm(xa) * (1.0 + mod_s[4, 0:1, :]) + mod_s[3, 0:1, :]
        return xa, hb

    u_s[:PAD, :] = jnp.zeros((PAD, D), F32)
    u_s[PAD + S:, :] = jnp.zeros((PAD, D), F32)

    def mix_in(i, carry):
        _, hb = resid(i)
        u = _gelu(_mm(_layernorm(hb).astype(BF16), w1_s[...]))
        u_s[pl.ds(pl.multiple_of(PAD + i * RB, 8), RB), :] = u
        return carry

    lax.fori_loop(0, n_chunk, mix_in, 0)

    def out_copy(i, slot):
        return pltpu.make_async_copy(
            out_s.at[slot], out_hbm.at[pl.ds(pl.multiple_of(i * RB, RB), RB), :],
            sem_out.at[slot])

    cq = D // 4

    def mlp(i, carry):
        slot = i % 2
        xa, hb = resid(i)
        win = pl.ds(pl.multiple_of(i * RB, 8), RB + 2 * PAD)
        parts = []
        for g, off in enumerate((-1, 1, -2, 2)):
            ug = u_s[win, g * cq:(g + 1) * cq]
            parts.append(ug[PAD + off:PAD + off + RB].astype(BF16))
        x1 = hb + _mm(jnp.concatenate(parts, axis=1), w2_s[...])
        t = _gelu(_mm(_layernorm(x1).astype(BF16), w3_s[...]))
        y = x1 + _mm(t.astype(BF16), w4_s[...])
        res = (xa + mod_s[5, 0:1, :] * y).astype(out_s.dtype)

        @pl.when(i >= 2)
        def _():
            out_copy(i - 2, slot).wait()

        out_s[slot] = res
        out_copy(i, slot).start()
        return carry

    lax.fori_loop(0, n_chunk, mlp, 0)
    out_copy(n_chunk - 2, (n_chunk - 2) % 2).wait()
    out_copy(n_chunk - 1, (n_chunk - 1) % 2).wait()


@functools.partial(jax.jit, static_argnames=("A_seg_len",))
def pallas_adaLN_cond__memory_aug_recurrent_mem_tr__mixer_s_mlp__prompt_kernel(
    A_x, A_mem0, A_Wq, A_Wk, A_Wv, A_Wo, A_seg_len,
    B_x, B_w1, B_w2, B_w3, B_w4, c, w_mod,
):
    del B_x
    B, S, D = A_x.shape
    _, H, Dh = A_Wq.shape
    M = A_mem0.shape[1]
    F = B_w3.shape[1]
    seg = int(A_seg_len)
    RB = 256
    assert B == 1 and Dh == LANES and S % RB == 0 and RB % seg == 0
    n_seg = S // seg

    hbm = pl.BlockSpec(memory_space=pl.ANY)
    vmem = pl.BlockSpec(memory_space=pltpu.VMEM)
    dma = pltpu.SemaphoreType.DMA

    out = pl.pallas_call(
        functools.partial(_kernel, S=S, D=D, H=H, Dh=Dh, M=M, seg=seg, F=F, RB=RB),
        out_shape=jax.ShapeDtypeStruct((S, D), A_x.dtype),
        in_specs=[hbm, vmem, hbm, hbm, hbm, hbm, hbm, hbm, hbm, hbm, vmem, hbm],
        out_specs=hbm,
        scratch_shapes=[
            pltpu.VMEM((S, D), A_x.dtype),
            pltpu.VMEM((n_seg + 1, M + seg, D), F32),
            pltpu.VMEM((3, H, D // 2, Dh), U32),
            pltpu.VMEM((D // LANES, H * Dh, LANES), BF16),
            pltpu.VMEM((2, D, HEAD_TILE, Dh), BF16),
            pltpu.VMEM((3, D, 2 * D), BF16),
            pltpu.VMEM((6, 8, D), F32),
            pltpu.VMEM((D, D), BF16),
            pltpu.VMEM((D, D), BF16),
            pltpu.VMEM((D, F), BF16),
            pltpu.VMEM((F, D), BF16),
            pltpu.VMEM((S + 16, D), F32),
            pltpu.VMEM((M + seg, H * Dh), F32),
            pltpu.VMEM((2, RB, D), A_x.dtype),
            dma(()), dma((2,)), dma((D // LANES,)), dma((3,)), dma((4,)), dma((2,)),
        ],
        compiler_params=pltpu.CompilerParams(vmem_limit_bytes=120 * 1024 * 1024),
    )(
        A_x.reshape(S, D), A_mem0.reshape(M, D), A_Wq, A_Wk, A_Wv,
        A_Wo.reshape(H * Dh, D), B_w1, B_w2, B_w3, B_w4, c, w_mod,
    )
    return out.reshape(B, S, D)
```

```python
import functools

import jax
import jax.numpy as jnp
from jax import lax
import jax.experimental.pallas as pl
import jax.experimental.pallas.tpu as pltpu

F32 = jnp.float32
BF16 = jnp.bfloat16
U32 = jnp.uint32
LANES = 128
SUB = 8
HEAD_TILE = 8
LAG_S = 1
LAG_PV = 4
N_PART = 8
EPS = 1e-5

_NN = (((1,), (0,)), ((), ()))
_NT = (((1,), (1,)), ((), ()))


def _mm(a, b, dims=_NN):
    return lax.dot_general(a, b, dims, preferred_element_type=F32)


def _bf(w):
    return pltpu.bitcast(w, BF16)


def _layernorm(x):
    m = jnp.mean(x, axis=-1, keepdims=True)
    d = x - m
    v = jnp.mean(d * d, axis=-1, keepdims=True)
    return d * lax.rsqrt(v + EPS)


def _gelu(x):
    k = 0.7978845608028654
    return (0.5 * x) * (1.0 + jnp.tanh(k * (x + 0.044715 * (x * x * x))))


def _kernel(
    x_hbm, mem0_ref, wq_hbm, wk_hbm, wv_hbm, wo_hbm,
    w1_hbm, w2_hbm, w3_hbm, w4_hbm, c_ref, wmod_hbm,
    out_hbm,
    x_s, hx, mod_s, w1_s, w2_s, w3_s, w4_s,
    sem_x, sem_stage, sem_wo, sem_mod, sem_b, sem_out,
    *, S, D, H, Dh, M, seg, F, RB,
):
    n_seg = S // seg
    L = M + seg
    n_col = D // LANES
    scale = Dh ** (-0.5)
    ride = seg - M
    ahead = S - n_seg * ride
    ring = ahead + seg
    n_ht = H // HEAD_TILE
    ln_rows = (S - ahead) // (3 * n_ht)

    b_copies = [
        pltpu.make_async_copy(src, dst, sem_b.at[i])
        for i, (src, dst) in enumerate(
            ((w1_hbm, w1_s), (w2_hbm, w2_s), (w3_hbm, w3_s), (w4_hbm, w4_s)))
    ]

    def attention(wq_s, wk_s, wv_s, wo_s, q_r, k_r, v_r, stage, wmod_s, hb_s, hc_s, *o_s):
        w_hbm = (wq_hbm, wk_hbm, wv_hbm)
        w_s = (wq_s, wk_s, wv_s)
        rings = (q_r, k_r, v_r)

        def mod_copy(j, slot):
            return pltpu.make_async_copy(
                wmod_hbm.at[:, pl.ds(j * D, D)], wmod_s.at[slot], sem_mod.at[slot])

        x_head = pltpu.make_async_copy(
            x_hbm.at[pl.ds(0, ahead)], x_s.at[pl.ds(0, ahead)], sem_x.at[0])
        x_tail = pltpu.make_async_copy(
            x_hbm.at[pl.ds(ahead, S - ahead)], x_s.at[pl.ds(ahead, S - ahead)], sem_x.at[1])

        def stage_copy(m, t):
            heads = pl.ds(pl.multiple_of(t * HEAD_TILE, HEAD_TILE), HEAD_TILE)
            return pltpu.make_async_copy(
                w_hbm[m].at[:, heads, :], stage.at[m], sem_stage.at[m])

        def wo_copy(j):
            return pltpu.make_async_copy(
                wo_hbm.at[:, pl.ds(j * LANES, LANES)], wo_s.at[j], sem_wo.at[j])

        stage_copy(0, 0).start()
        mod_copy(0, 0).start()
        mod_copy(1, 1).start()
        x_head.start()
        stage_copy(1, 0).start()
        x_tail.start()
        stage_copy(2, 0).start()

        cv = c_ref[...].astype(F32)
        silu_c = jnp.broadcast_to(cv * (1.0 / (1.0 + jnp.exp(-cv))), (SUB, D))

        def make_mod(j, slot):
            mod_copy(j, slot).wait()
            mod_s[j] = _mm(silu_c, wmod_s[slot])

        def retile(m, t, pieces=range(D // 64)):
            for r in pieces:
                blk = jnp.transpose(stage[m, r * 64:(r + 1) * 64, :, :], (1, 0, 2))
                for hh in range(HEAD_TILE):
                    w_s[m][t * HEAD_TILE + hh, r * 32:(r + 1) * 32, :] = (
                        pltpu.bitcast(blk[hh], U32))

        def modulate(start, n):
            rows = pl.ds(pl.multiple_of(start, 16), n)
            return rows, (_layernorm(x_s[rows, :].astype(F32))
                          * (1.0 + mod_s[1, 0:1, :]) + mod_s[0, 0:1, :])

        stage_copy(0, 0).wait()
        retile(0, 0)
        stage_copy(0, 1).start()
        make_mod(0, 0)
        make_mod(1, 1)
        mod_copy(2, 0).start()
        mod_copy(3, 1).start()
        for j in range(n_col):
            wo_copy(j).start()
        x_head.wait()

        def head_rows(i, carry):
            rows, hv = modulate(i * 64, 64)
            hb_s[rows, :] = hv.astype(BF16)
            return carry

        lax.fori_loop(0, ahead // 64, head_rows, 0, unroll=2)
        x_tail.wait()

        def bulk(t, carry):
            for m in range(3):
                nm, nt = (m + 1) % 3, t + (m + 1) // 3
                if m < 2:
                    stage_copy(nm, nt).wait()
                else:
                    nt = jnp.minimum(nt, n_ht - 1)

                    @pl.when(t + 1 < n_ht)
                    def _():
                        stage_copy(nm, nt).wait()

                lr, pc = ln_rows // HEAD_TILE, D // 64 // HEAD_TILE
                for hh in range(HEAD_TILE):
                    h = t * HEAD_TILE + hh
                    rings[m][h, :ahead, :] = _mm(hb_s[...], _bf(w_s[m][h]))
                    retile(nm, nt, range(hh * pc, (hh + 1) * pc))
                    rows, hv = modulate(ahead + (3 * t + m) * ln_rows + hh * lr, lr)
                    hx[rows, :] = hv

                @pl.when(nt + 1 < n_ht)
                def _():
                    stage_copy(nm, nt + 1).start()

            return carry

        lax.fori_loop(0, n_ht, bulk, 0)

        make_mod(2, 0)
        make_mod(3, 1)
        mod_copy(4, 0).start()
        mod_copy(5, 1).start()
        for cp in b_copies:
            cp.start()
        for j in range(n_col):
            wo_copy(j).wait()

        hc_s[:M, :] = mem0_ref[...].astype(F32)
        hc_s[M:, :] = hx[ahead:ahead + ride, :]

        row = lax.broadcasted_iota(jnp.int32, (L, L), 0)
        col = lax.broadcasted_iota(jnp.int32, (L, L), 1)
        mask = (row < M) | (row >= col)
        hpp = H // N_PART
        part = hpp * Dh

        def step(s, carry):
            rd = pl.ds(pl.multiple_of(lax.rem(s * seg, ring), SUB), seg)
            wr = [pl.ds(pl.multiple_of(lax.rem(ahead + s * ride + j * SUB, ring), SUB), SUB)
                  for j in range(ride // SUB)]
            qkv, ev = {}, {}
            acc = [None] * n_col

            def project(p):
                ks = slice(p * part, (p + 1) * part)
                for j in range(n_col):
                    r = _mm(o_s[p][...], wo_s[j, ks, :])
                    acc[j] = r if acc[j] is None else acc[j] + r

            for t in range(H + max(LAG_PV, N_PART)):
                if 0 <= t - LAG_S < H:
                    h = t - LAG_S
                    q, k, v = (jnp.concatenate([pm, r_[h, rd, :]], axis=0)
                               for pm, r_ in zip(qkv.pop(h), rings))
                if t < H:
                    res = [_mm(hc_s[...], _bf(w[t])) for w in w_s]
                    for r, r_ in zip(res, rings):
                        for j, rows in enumerate(wr):
                            r_[t, rows, :] = r[M + j * SUB:M + (j + 1) * SUB]
                    qkv[t] = [r[:M] for r in res]
                else:
                    project(t - H)
                if 0 <= t - LAG_S < H:
                    sc = jnp.where(mask, _mm(q, k.astype(BF16), _NT) * scale, -1000000000.0)
                    e = jnp.exp(sc - jnp.max(sc, axis=-1, keepdims=True))
                    ev[t - LAG_S] = (e / jnp.sum(e, axis=-1, keepdims=True), v.astype(BF16))
                if 0 <= t - LAG_PV < H:
                    h = t - LAG_PV
                    o_s[h // hpp][:, (h % hpp) * Dh:(h % hpp + 1) * Dh] = _mm(*ev.pop(h))
            nxt = jnp.minimum(ahead + (s + 1) * ride, S - ride)
            hc_s[M:, :] = hx[pl.ds(pl.multiple_of(nxt, SUB), ride), :]
            rows = pl.ds(pl.multiple_of(s * seg, seg), seg)
            for j in range(n_col):
                cols = slice(j * LANES, (j + 1) * LANES)
                hc_s[:M, cols] = acc[j][:M]
                hx[rows, cols] = x_s[rows, cols].astype(F32) + mod_s[2, 0:1, cols] * acc[j][M:]
            return carry

        lax.fori_loop(0, n_seg, step, 0)
        make_mod(4, 0)
        make_mod(5, 1)

    pl.run_scoped(
        attention,
        pltpu.VMEM((H, D // 2, Dh), U32),
        pltpu.VMEM((H, D // 2, Dh), U32),
        pltpu.VMEM((H, D // 2, Dh), U32),
        pltpu.VMEM((n_col, H * Dh, LANES), BF16),
        pltpu.VMEM((H, ring, Dh), F32),
        pltpu.VMEM((H, ring, Dh), F32),
        pltpu.VMEM((H, ring, Dh), F32),
        pltpu.VMEM((3, D, HEAD_TILE, Dh), BF16),
        pltpu.VMEM((2, D, D), BF16),
        pltpu.VMEM((ahead, D), BF16),
        pltpu.VMEM((seg, D), F32),
        *[pltpu.VMEM((L, H * Dh // N_PART), F32)] * N_PART,
    )

    def mixer(u_s, out_s):
        PAD = SUB
        n_chunk = S // RB
        for cp in b_copies:
            cp.wait()

        def resid(i):
            xa = hx[pl.ds(pl.multiple_of(i * RB, RB), RB), :]
            return xa, _layernorm(xa) * (1.0 + mod_s[4, 0:1, :]) + mod_s[3, 0:1, :]

        u_s[:PAD, :] = jnp.zeros((PAD, D), F32)
        u_s[PAD + S:, :] = jnp.zeros((PAD, D), F32)

        def mix_in(i, carry):
            _, hb = resid(i)
            u = _gelu(_mm(_layernorm(hb).astype(BF16), w1_s[...]))
            u_s[pl.ds(pl.multiple_of(PAD + i * RB, 8), RB), :] = u
            return carry

        lax.fori_loop(0, n_chunk, mix_in, 0)

        def out_copy(i, slot):
            return pltpu.make_async_copy(
                out_s.at[slot], out_hbm.at[pl.ds(pl.multiple_of(i * RB, RB), RB), :],
                sem_out.at[slot])

        cq = D // 4

        def mlp(i, carry):
            slot = i % 2
            xa, hb = resid(i)
            win = pl.ds(pl.multiple_of(i * RB, 8), RB + 2 * PAD)
            parts = []
            for g, off in enumerate((-1, 1, -2, 2)):
                ug = u_s[win, g * cq:(g + 1) * cq]
                parts.append(ug[PAD + off:PAD + off + RB].astype(BF16))
            x1 = hb + _mm(jnp.concatenate(parts, axis=1), w2_s[...])
            t = _gelu(_mm(_layernorm(x1).astype(BF16), w3_s[...]))
            y = x1 + _mm(t.astype(BF16), w4_s[...])
            res = (xa + mod_s[5, 0:1, :] * y).astype(out_s.dtype)

            @pl.when(i >= 2)
            def _():
                out_copy(i - 2, slot).wait()

            out_s[slot] = res
            out_copy(i, slot).start()
            return carry

        lax.fori_loop(0, n_chunk, mlp, 0)
        out_copy(n_chunk - 2, (n_chunk - 2) % 2).wait()
        out_copy(n_chunk - 1, (n_chunk - 1) % 2).wait()

    pl.run_scoped(
        mixer,
        pltpu.VMEM((S + 2 * SUB, D), F32),
        pltpu.VMEM((2, RB, D), out_hbm.dtype),
    )


@functools.partial(jax.jit, static_argnames=("A_seg_len",))
def pallas_adaLN_cond__memory_aug_recurrent_mem_tr__mixer_s_mlp__prompt_kernel(
    A_x, A_mem0, A_Wq, A_Wk, A_Wv, A_Wo, A_seg_len,
    B_x, B_w1, B_w2, B_w3, B_w4, c, w_mod,
):
    del B_x
    B, S, D = A_x.shape
    _, H, Dh = A_Wq.shape
    M = A_mem0.shape[1]
    F = B_w3.shape[1]
    seg = int(A_seg_len)
    RB = 256
    assert B == 1 and Dh == LANES and S % RB == 0 and RB % seg == 0

    hbm = pl.BlockSpec(memory_space=pl.ANY)
    vmem = pl.BlockSpec(memory_space=pltpu.VMEM)
    dma = pltpu.SemaphoreType.DMA

    out = pl.pallas_call(
        functools.partial(_kernel, S=S, D=D, H=H, Dh=Dh, M=M, seg=seg, F=F, RB=RB),
        out_shape=jax.ShapeDtypeStruct((S, D), A_x.dtype),
        in_specs=[hbm, vmem, hbm, hbm, hbm, hbm, hbm, hbm, hbm, hbm, vmem, hbm],
        out_specs=hbm,
        scratch_shapes=[
            pltpu.VMEM((S, D), A_x.dtype),
            pltpu.VMEM((S, D), F32),
            pltpu.VMEM((6, SUB, D), F32),
            pltpu.VMEM((D, D), BF16),
            pltpu.VMEM((D, D), BF16),
            pltpu.VMEM((D, F), BF16),
            pltpu.VMEM((F, D), BF16),
            dma((2,)), dma((3,)), dma((D // LANES,)), dma((2,)), dma((4,)), dma((2,)),
        ],
        compiler_params=pltpu.CompilerParams(vmem_limit_bytes=124 * 1024 * 1024),
    )(
        A_x.reshape(S, D), A_mem0.reshape(M, D), A_Wq, A_Wk, A_Wv,
        A_Wo.reshape(H * Dh, D), B_w1, B_w2, B_w3, B_w4, c, w_mod,
    )
    return out.reshape(B, S, D)
```

```python
import functools

import jax
import jax.numpy as jnp
from jax import lax
import jax.experimental.pallas as pl
import jax.experimental.pallas.tpu as pltpu

F32 = jnp.float32
BF16 = jnp.bfloat16
U32 = jnp.uint32
LANES = 128
SUB = 8
HEAD_TILE = 8
LAG_S = 1
LAG_PV = 4
N_PART = 8
EPS = 1e-5

_NN = (((1,), (0,)), ((), ()))
_NT = (((1,), (1,)), ((), ()))


def _mm(a, b, dims=_NN):
    return lax.dot_general(a, b, dims, preferred_element_type=F32)


def _bf(w):
    return pltpu.bitcast(w, BF16)


def _layernorm(x):
    m = jnp.mean(x, axis=-1, keepdims=True)
    d = x - m
    v = jnp.mean(d * d, axis=-1, keepdims=True)
    return d * lax.rsqrt(v + EPS)


def _gelu(x):
    k = 0.7978845608028654
    return (0.5 * x) * (1.0 + jnp.tanh(k * (x + 0.044715 * (x * x * x))))


def _kernel(
    x_hbm, mem0_ref, wq_hbm, wk_hbm, wv_hbm, wo_hbm,
    w1_hbm, w2_hbm, w3_hbm, w4_hbm, c_ref, wmod_hbm,
    out_hbm,
    x_s, hx, mod_s, w1_s, w2_s, w3_s, w4_s,
    sem_x, sem_stage, sem_wo, sem_mod, sem_b, sem_out,
    *, S, D, H, Dh, M, seg, F, RB,
):
    n_seg = S // seg
    L = M + seg
    n_col = D // LANES
    scale = Dh ** (-0.5)
    ride = seg - M
    ahead = S - n_seg * ride
    ring = ahead + seg
    n_ht = H // HEAD_TILE

    b_copies = [
        pltpu.make_async_copy(src, dst, sem_b.at[i])
        for i, (src, dst) in enumerate(
            ((w1_hbm, w1_s), (w2_hbm, w2_s), (w3_hbm, w3_s), (w4_hbm, w4_s)))
    ]

    def attention(w_s, wo_s, qkv_r, stage, wmod_s, hc_s, *o_s):
        w_hbm = (wq_hbm, wk_hbm, wv_hbm)
        n_w = 3 * n_ht

        def slot(m, h):
            return (3 * (h // HEAD_TILE) + m) * HEAD_TILE + h % HEAD_TILE

        def mod_copy(j, b):
            return pltpu.make_async_copy(
                wmod_hbm.at[:, pl.ds(j * D, D)], wmod_s.at[b], sem_mod.at[b])

        x_head = pltpu.make_async_copy(
            x_hbm.at[pl.ds(0, ahead)], x_s.at[pl.ds(0, ahead)], sem_x.at[0])
        x_tail = pltpu.make_async_copy(
            x_hbm.at[pl.ds(ahead, S - ahead)], x_s.at[pl.ds(ahead, S - ahead)], sem_x.at[1])

        def stage_copy(m, t):
            heads = pl.ds(pl.multiple_of(t * HEAD_TILE, HEAD_TILE), HEAD_TILE)
            return pltpu.make_async_copy(
                w_hbm[m].at[:, heads, :], stage.at[m], sem_stage.at[m])

        def wo_copy(j):
            cols = pl.ds(pl.multiple_of(j * LANES, LANES), LANES)
            return pltpu.make_async_copy(wo_hbm.at[:, cols], wo_s.at[j], sem_wo.at[j])

        stage_copy(0, 0).start()
        mod_copy(0, 0).start()
        mod_copy(1, 1).start()
        x_head.start()

        cv = c_ref[...].astype(F32)
        silu_c = jnp.broadcast_to(cv * (1.0 / (1.0 + jnp.exp(-cv))), (SUB, D))

        def make_mod(j, b):
            mod_copy(j, b).wait()
            mod_s[j] = _mm(silu_c, wmod_s[b])

        def retile(i, pieces=range(D // 64)):
            src = lax.rem(i, 3)
            for r in pieces:
                blk = jnp.transpose(stage[src, r * 64:(r + 1) * 64, :, :], (1, 0, 2))
                for hh in range(HEAD_TILE):
                    w_s[i * HEAD_TILE + hh, r * 32:(r + 1) * 32, :] = (
                        pltpu.bitcast(blk[hh], U32))

        def modulate(start, n):
            rows = pl.ds(pl.multiple_of(start, SUB), n)
            return (_layernorm(x_s[rows, :].astype(F32))
                    * (1.0 + mod_s[1, 0:1, :]) + mod_s[0, 0:1, :])

        stage_copy(0, 0).wait()
        stage_copy(1, 0).start()
        retile(0)
        make_mod(0, 0)
        make_mod(1, 1)
        x_head.wait()
        stage_copy(2, 0).start()

        def head_rows(i, carry):
            hx[pl.ds(pl.multiple_of(i * 64, 64), 64), :] = modulate(i * 64, 64)
            return carry

        lax.fori_loop(0, ahead // 64, head_rows, 0, unroll=2)

        def bulk(i, carry):
            nxt = jnp.minimum(i + 1, n_w - 1)
            for m in range(3):
                @pl.when((i + 3 < n_w) & (lax.rem(i, 3) == m))
                def _():
                    stage_copy(m, i // 3 + 1).start()

                @pl.when((i + 1 < n_w) & (lax.rem(i + 1, 3) == m))
                def _():
                    stage_copy(m, (i + 1) // 3).wait()

            @pl.when(i < n_col)
            def _():
                wo_copy(i).start()

            @pl.when(i == n_col + 2)
            def _():
                x_tail.start()

            for j in range(2):
                @pl.when(i == n_col + j)
                def _():
                    mod_copy(2 + j, j).start()

            pc = D // 64 // HEAD_TILE
            for hh in range(HEAD_TILE):
                j = i * HEAD_TILE + hh
                qkv_r[j, :ahead, :] = _mm(hx[:ahead, :], _bf(w_s[j]))
                retile(nxt, range(hh * pc, (hh + 1) * pc))
            return carry

        lax.fori_loop(0, n_w, bulk, 0)

        make_mod(2, 0)
        make_mod(3, 1)
        mod_copy(4, 0).start()
        mod_copy(5, 1).start()
        for cp in b_copies:
            cp.start()
        for j in range(n_col):
            wo_copy(j).wait()

        hc_s[:M, :] = mem0_ref[...].astype(F32)
        x_tail.wait()
        hc_s[M:, :] = modulate(ahead, ride)

        row = lax.broadcasted_iota(jnp.int32, (L, L), 0)
        col = lax.broadcasted_iota(jnp.int32, (L, L), 1)
        mask = (row < M) | (row >= col)
        hpp = H // N_PART
        part = hpp * Dh

        def step(s, carry):
            rd = pl.ds(pl.multiple_of(lax.rem(s * seg, ring), SUB), seg)
            wr = [pl.ds(pl.multiple_of(lax.rem(ahead + s * ride + j * SUB, ring), SUB), SUB)
                  for j in range(ride // SUB)]
            qkv, ev = {}, {}
            acc = [None] * n_col

            def project(p):
                ks = slice(p * part, (p + 1) * part)
                for j in range(n_col):
                    r = _mm(o_s[p][...], wo_s[j, ks, :])
                    acc[j] = r if acc[j] is None else acc[j] + r

            for t in range(H + max(LAG_PV, N_PART)):
                if 0 <= t - LAG_S < H:
                    h = t - LAG_S
                    q, k, v = (jnp.concatenate([pm, qkv_r[slot(m, h), rd, :]], axis=0)
                               for m, pm in enumerate(qkv.pop(h)))
                if t < H:
                    res = [_mm(hc_s[...], _bf(w_s[slot(m, t)])) for m in range(3)]
                    for m, r in enumerate(res):
                        for j, rows in enumerate(wr):
                            qkv_r[slot(m, t), rows, :] = r[M + j * SUB:M + (j + 1) * SUB]
                    qkv[t] = [r[:M] for r in res]
                else:
                    project(t - H)
                if 0 <= t - LAG_S < H:
                    sc = jnp.where(mask, _mm(q, k.astype(BF16), _NT) * scale, -1000000000.0)
                    e = jnp.exp(sc - jnp.max(sc, axis=-1, keepdims=True))
                    ev[t - LAG_S] = (e / jnp.sum(e, axis=-1, keepdims=True), v.astype(BF16))
                if 0 <= t - LAG_PV < H:
                    h = t - LAG_PV
                    o_s[h // hpp][:, (h % hpp) * Dh:(h % hpp + 1) * Dh] = _mm(*ev.pop(h))
            nxt = jnp.minimum(ahead + (s + 1) * ride, S - ride)
            hc_s[M:, :] = modulate(nxt, ride)
            rows = pl.ds(pl.multiple_of(s * seg, seg), seg)
            for j in range(n_col):
                cols = slice(j * LANES, (j + 1) * LANES)
                hc_s[:M, cols] = acc[j][:M]
                hx[rows, cols] = x_s[rows, cols].astype(F32) + mod_s[2, 0:1, cols] * acc[j][M:]
            return carry

        lax.fori_loop(0, n_seg, step, 0)
        make_mod(4, 0)
        make_mod(5, 1)

    pl.run_scoped(
        attention,
        pltpu.VMEM((3 * H, D // 2, Dh), U32),
        pltpu.VMEM((n_col, H * Dh, LANES), BF16),
        pltpu.VMEM((3 * H, ring, Dh), F32),
        pltpu.VMEM((3, D, HEAD_TILE, Dh), BF16),
        pltpu.VMEM((2, D, D), BF16),
        pltpu.VMEM((seg, D), F32),
        *[pltpu.VMEM((L, H * Dh // N_PART), F32)] * N_PART,
    )

    def mixer(u_s, out_s):
        PAD = SUB
        n_chunk = S // RB
        for cp in b_copies:
            cp.wait()

        def resid(i):
            xa = hx[pl.ds(pl.multiple_of(i * RB, RB), RB), :]
            return xa, _layernorm(xa) * (1.0 + mod_s[4, 0:1, :]) + mod_s[3, 0:1, :]

        u_s[:PAD, :] = jnp.zeros((PAD, D), F32)
        u_s[PAD + S:, :] = jnp.zeros((PAD, D), F32)

        def mix_in(i, carry):
            _, hb = resid(i)
            u = _gelu(_mm(_layernorm(hb), w1_s[...]))
            u_s[pl.ds(pl.multiple_of(PAD + i * RB, 8), RB), :] = u
            return carry

        lax.fori_loop(0, n_chunk, mix_in, 0)

        def out_copy(i, slot):
            return pltpu.make_async_copy(
                out_s.at[slot], out_hbm.at[pl.ds(pl.multiple_of(i * RB, RB), RB), :],
                sem_out.at[slot])

        cq = D // 4

        def mlp(i, carry):
            slot = i % 2
            xa, hb = resid(i)
            win = pl.ds(pl.multiple_of(i * RB, 8), RB + 2 * PAD)
            parts = []
            for g, off in enumerate((-1, 1, -2, 2)):
                ug = u_s[win, g * cq:(g + 1) * cq]
                parts.append(ug[PAD + off:PAD + off + RB])
            x1 = hb + _mm(jnp.concatenate(parts, axis=1), w2_s[...])
            t = _gelu(_mm(_layernorm(x1), w3_s[...]))
            y = x1 + _mm(t, w4_s[...])
            res = (xa + mod_s[5, 0:1, :] * y).astype(out_s.dtype)

            @pl.when(i >= 2)
            def _():
                out_copy(i - 2, slot).wait()

            out_s[slot] = res
            out_copy(i, slot).start()
            return carry

        lax.fori_loop(0, n_chunk, mlp, 0)
        out_copy(n_chunk - 2, (n_chunk - 2) % 2).wait()
        out_copy(n_chunk - 1, (n_chunk - 1) % 2).wait()

    pl.run_scoped(
        mixer,
        pltpu.VMEM((S + 2 * SUB, D), F32),
        pltpu.VMEM((2, RB, D), out_hbm.dtype),
    )


@functools.partial(jax.jit, static_argnames=("A_seg_len",))
def pallas_adaLN_cond__memory_aug_recurrent_mem_tr__mixer_s_mlp__prompt_kernel(
    A_x, A_mem0, A_Wq, A_Wk, A_Wv, A_Wo, A_seg_len,
    B_x, B_w1, B_w2, B_w3, B_w4, c, w_mod,
):
    del B_x
    B, S, D = A_x.shape
    _, H, Dh = A_Wq.shape
    M = A_mem0.shape[1]
    F = B_w3.shape[1]
    seg = int(A_seg_len)
    RB = 256
    assert B == 1 and Dh == LANES and S % RB == 0 and RB % seg == 0

    hbm = pl.BlockSpec(memory_space=pl.ANY)
    vmem = pl.BlockSpec(memory_space=pltpu.VMEM)
    dma = pltpu.SemaphoreType.DMA

    out = pl.pallas_call(
        functools.partial(_kernel, S=S, D=D, H=H, Dh=Dh, M=M, seg=seg, F=F, RB=RB),
        out_shape=jax.ShapeDtypeStruct((S, D), A_x.dtype),
        in_specs=[hbm, vmem, hbm, hbm, hbm, hbm, hbm, hbm, hbm, hbm, vmem, hbm],
        out_specs=hbm,
        scratch_shapes=[
            pltpu.VMEM((S, D), A_x.dtype),
            pltpu.VMEM((S, D), F32),
            pltpu.VMEM((6, SUB, D), F32),
            pltpu.VMEM((D, D), BF16),
            pltpu.VMEM((D, D), BF16),
            pltpu.VMEM((D, F), BF16),
            pltpu.VMEM((F, D), BF16),
            dma((2,)), dma((3,)), dma((D // LANES,)), dma((2,)), dma((4,)), dma((2,)),
        ],
        compiler_params=pltpu.CompilerParams(vmem_limit_bytes=124 * 1024 * 1024),
    )(
        A_x.reshape(S, D), A_mem0.reshape(M, D), A_Wq, A_Wk, A_Wv,
        A_Wo.reshape(H * Dh, D), B_w1, B_w2, B_w3, B_w4, c, w_mod,
    )
    return out.reshape(B, S, D)
```

```python
import functools

import jax
import jax.numpy as jnp
from jax import lax
import jax.experimental.pallas as pl
import jax.experimental.pallas.tpu as pltpu

F32 = jnp.float32
BF16 = jnp.bfloat16
U32 = jnp.uint32
LANES = 128
SUB = 8
HEAD_TILE = 8
LAG_S = 1
LAG_PV = 4
LAG_V = 2
OUT_T0 = 30
MIX_T = 31
N_PART = 8
N_SPLIT = 2
ROWS = 256
EPS = 1e-5

_NN = (((1,), (0,)), ((), ()))
_NT = (((1,), (1,)), ((), ()))


def _mm(a, b, dims=_NN):
    return lax.dot_general(a, b, dims, preferred_element_type=F32)


def _bf(w):
    return pltpu.bitcast(w, BF16)


def _layernorm(x):
    m = jnp.mean(x, axis=-1, keepdims=True)
    d = x - m
    v = jnp.mean(d * d, axis=-1, keepdims=True)
    return d * lax.rsqrt(v + EPS)


def _gelu(x):
    k = 0.7978845608028654
    return (0.5 * x) * (1.0 + jnp.tanh(k * (x + 0.044715 * (x * x * x))))


def _kernel(
    x_hbm, mem0_ref, wq_hbm, wk_hbm, wv_hbm, wo_hbm,
    w1_hbm, w2_hbm, w3_hbm, w4_hbm, c_ref, wmod_hbm,
    out_hbm,
    x_s, hx, u_s, mod_s, w2_s, w3_s, w4_s,
    sem_x, sem_stage, sem_wo, sem_w1, sem_mod, sem_b, sem_out,
    *, S, D, H, Dh, M, seg, F, RB,
):
    n_seg = S // seg
    L = M + seg
    n_col = D // LANES
    scale = Dh ** (-0.5)
    ride = seg - M
    ahead = S - n_seg * ride
    ring = ahead + seg
    n_ht = H // HEAD_TILE

    b_copies = [
        pltpu.make_async_copy(src, dst, sem_b.at[i])
        for i, (src, dst) in enumerate(
            ((w2_hbm, w2_s), (w3_hbm, w3_s), (w4_hbm, w4_s)))
    ]

    PAD = SUB
    u_s[:PAD, :] = jnp.zeros((PAD, D), F32)
    u_s[PAD + S:, :] = jnp.zeros((PAD, D), F32)

    def cond(xa):
        return _layernorm(xa) * (1.0 + mod_s[4, 0:1, :]) + mod_s[3, 0:1, :]

    def attention(w_s, wo_s, w1_s, qkv_r, stage, wmod_s, hc_s, *o_s):
        w_hbm = (wq_hbm, wk_hbm, wv_hbm)
        n_w = 3 * n_ht

        def slot(m, h):
            return (3 * (h // HEAD_TILE) + m) * HEAD_TILE + h % HEAD_TILE

        def mod_copy(j, b):
            return pltpu.make_async_copy(
                wmod_hbm.at[:, pl.ds(j * D, D)], wmod_s.at[b], sem_mod.at[b])

        x_head = pltpu.make_async_copy(
            x_hbm.at[pl.ds(0, ahead)], x_s.at[pl.ds(0, ahead)], sem_x.at[0])
        x_tail = pltpu.make_async_copy(
            x_hbm.at[pl.ds(ahead, S - ahead)], x_s.at[pl.ds(ahead, S - ahead)], sem_x.at[1])

        def stage_copy(m, t):
            heads = pl.ds(pl.multiple_of(t * HEAD_TILE, HEAD_TILE), HEAD_TILE)
            return pltpu.make_async_copy(
                w_hbm[m].at[:, heads, :], stage.at[m], sem_stage.at[m])

        def wo_copy(j):
            cols = pl.ds(pl.multiple_of(j * LANES, LANES), LANES)
            return (pltpu.make_async_copy(wo_hbm.at[:, cols], wo_s.at[j], sem_wo.at[j]),
                    pltpu.make_async_copy(w1_hbm.at[:, cols], w1_s.at[j], sem_w1.at[j]))

        stage_copy(0, 0).start()
        mod_copy(0, 0).start()
        mod_copy(1, 1).start()
        x_head.start()

        cv = c_ref[...].astype(F32)
        silu_c = jnp.broadcast_to(cv * (1.0 / (1.0 + jnp.exp(-cv))), (SUB, D))

        def make_mod(j, b):
            mod_copy(j, b).wait()
            mod_s[j] = _mm(silu_c, wmod_s[b])

        def retile(i, pieces=range(D // 64)):
            src = lax.rem(i, 3)
            for r in pieces:
                blk = jnp.transpose(stage[src, r * 64:(r + 1) * 64, :, :], (1, 0, 2))
                for hh in range(HEAD_TILE):
                    w_s[i * HEAD_TILE + hh, r * 32:(r + 1) * 32, :] = (
                        pltpu.bitcast(blk[hh], U32))

        def modulate(start, n):
            rows = pl.ds(pl.multiple_of(start, SUB), n)
            return (_layernorm(x_s[rows, :].astype(F32))
                    * (1.0 + mod_s[1, 0:1, :]) + mod_s[0, 0:1, :])

        stage_copy(0, 0).wait()
        stage_copy(1, 0).start()
        retile(0)
        make_mod(0, 0)
        make_mod(1, 1)
        x_head.wait()
        stage_copy(2, 0).start()

        def head_rows(i, carry):
            hx[pl.ds(pl.multiple_of(i * 64, 64), 64), :] = modulate(i * 64, 64)
            return carry

        lax.fori_loop(0, ahead // 64, head_rows, 0, unroll=2)

        def bulk(i, carry):
            nxt = jnp.minimum(i + 1, n_w - 1)
            for m in range(3):
                @pl.when((i + 3 < n_w) & (lax.rem(i, 3) == m))
                def _():
                    stage_copy(m, i // 3 + 1).start()

                @pl.when((i + 1 < n_w) & (lax.rem(i + 1, 3) == m))
                def _():
                    stage_copy(m, (i + 1) // 3).wait()

            @pl.when(i < n_col)
            def _():
                for cp in wo_copy(i):
                    cp.start()

            @pl.when(i == n_col + 1)
            def _():
                x_tail.start()

            for j in range(4):
                @pl.when(i == n_col - 1 + j)
                def _():
                    mod_copy(2 + j, j).start()

            pc = D // 64 // HEAD_TILE
            for hh in range(HEAD_TILE):
                j = i * HEAD_TILE + hh
                qkv_r[j, :ahead, :] = _mm(hx[:ahead, :], _bf(w_s[j]))
                retile(nxt, range(hh * pc, (hh + 1) * pc))
            return carry

        lax.fori_loop(0, n_w, bulk, 0)

        for j in range(4):
            make_mod(2 + j, j)
        for cp in b_copies:
            cp.start()
        for j in range(n_col):
            for cp in wo_copy(j):
                cp.wait()

        hc_s[:M, :] = mem0_ref[...].astype(F32)
        x_tail.wait()
        hc_s[M:, :] = modulate(ahead, ride)

        row = lax.broadcasted_iota(jnp.int32, (L, L), 0)
        col = lax.broadcasted_iota(jnp.int32, (L, L), 1)
        mask = (row < M) | (row >= col)
        hpp = H // N_PART
        part = hpp * Dh

        def mix_in(s):
            start = pl.multiple_of(s * seg, seg)
            z = _layernorm(cond(hx[pl.ds(start, seg), :]))
            for j in range(n_col):
                u_s[pl.ds(start + PAD, seg), j * LANES:(j + 1) * LANES] = _gelu(_mm(z, w1_s[j]))

        def step(s, carry):
            rd = pl.ds(pl.multiple_of(lax.rem(s * seg, ring), SUB), seg)
            wr = [pl.ds(pl.multiple_of(lax.rem(ahead + s * ride + j * SUB, ring), SUB), SUB)
                  for j in range(ride // SUB)]
            qkv, ev = {}, {}
            acc = [None] * n_col

            def project(p):
                ks = slice(p * part, (p + 1) * part)
                for j in range(n_col):
                    r = _mm(o_s[p][...], wo_s[j, ks, :])
                    acc[j] = r if acc[j] is None else acc[j] + r

            def project_in(m, h):
                r = _mm(hc_s[...], _bf(w_s[slot(m, h)]))
                for j, rows in enumerate(wr):
                    qkv_r[slot(m, h), rows, :] = r[M + j * SUB:M + (j + 1) * SUB]
                qkv[m, h] = r[:M]

            def gather(m, h):
                return jnp.concatenate([qkv.pop((m, h)), qkv_r[slot(m, h), rd, :]], axis=0)

            n_out = 0
            for t in range(H + LAG_PV):
                hs, hp = t - LAG_S, t - LAG_PV
                if 0 <= hs < H:
                    q, k = gather(0, hs), gather(1, hs).astype(BF16)
                if 0 <= hp < H:
                    v = gather(2, hp).astype(BF16)
                if t < H:
                    project_in(0, t)
                    project_in(1, t)
                if 0 <= t - LAG_V < H:
                    project_in(2, t - LAG_V)
                if t >= OUT_T0 and n_out < N_PART and (n_out + 1) * hpp <= hp:
                    project(n_out)
                    n_out += 1
                if t == MIX_T:
                    mix_in(jnp.maximum(s - 1, 0))
                if 0 <= hs < H:
                    sc = jnp.where(mask, _mm(q, k, _NT) * scale, -1000000000.0)
                    e = jnp.exp(sc - jnp.max(sc, axis=-1, keepdims=True))
                    ev[hs] = e / jnp.sum(e, axis=-1, keepdims=True)
                if 0 <= hp < H:
                    o_s[hp // hpp][:, (hp % hpp) * Dh:(hp % hpp + 1) * Dh] = _mm(ev.pop(hp), v)
            for p in range(n_out, N_PART):
                project(p)
            nxt = jnp.minimum(ahead + (s + 1) * ride, S - ride)
            hc_s[M:, :] = modulate(nxt, ride)
            rows = pl.ds(pl.multiple_of(s * seg, seg), seg)
            for j in range(n_col):
                cols = slice(j * LANES, (j + 1) * LANES)
                hc_s[:M, cols] = acc[j][:M]
                hx[rows, cols] = x_s[rows, cols].astype(F32) + mod_s[2, 0:1, cols] * acc[j][M:]
            return carry

        lax.fori_loop(0, n_seg, step, 0)
        mix_in(n_seg - 1)

    pl.run_scoped(
        attention,
        pltpu.VMEM((3 * H, D // 2, Dh), U32),
        pltpu.VMEM((n_col, H * Dh, LANES), BF16),
        pltpu.VMEM((n_col, D, LANES), BF16),
        pltpu.VMEM((3 * H, ring, Dh), F32),
        pltpu.VMEM((3, D, HEAD_TILE, Dh), BF16),
        pltpu.VMEM((4, D, D), BF16),
        pltpu.VMEM((seg, D), F32),
        *[pltpu.VMEM((L, H * Dh // N_PART), F32)] * N_PART,
    )

    def mixer(out_s):
        n_chunk = S // RB
        for cp in b_copies:
            cp.wait()

        def out_copy(i, slot):
            return pltpu.make_async_copy(
                out_s.at[slot], out_hbm.at[pl.ds(pl.multiple_of(i * RB, RB), RB), :],
                sem_out.at[slot])

        cq = D // 4

        def mlp(i, carry):
            slot = i % 2

            @pl.when(i >= 2)
            def _():
                out_copy(i - 2, slot).wait()

            rs = RB // N_SPLIT
            x1, t = [], []
            for a in range(N_SPLIT):
                start = pl.multiple_of(i * RB + a * rs, rs)
                parts = []
                for g, off in enumerate((-1, 1, -2, 2)):
                    ug = u_s[pl.ds(start, rs + 2 * PAD), g * cq:(g + 1) * cq]
                    parts.append(ug[PAD + off:PAD + off + rs])
                x1.append(cond(hx[pl.ds(start, rs), :])
                          + _mm(jnp.concatenate(parts, axis=1), w2_s[...]))
            for a in range(N_SPLIT):
                t.append(_gelu(_mm(_layernorm(x1[a]), w3_s[...])))
            for a in range(N_SPLIT):
                start = pl.multiple_of(i * RB + a * rs, rs)
                y = x1[a] + _mm(t[a], w4_s[...])
                out_s[slot, a * rs:(a + 1) * rs, :] = (
                    hx[pl.ds(start, rs), :] + mod_s[5, 0:1, :] * y).astype(out_s.dtype)
            out_copy(i, slot).start()
            return carry

        lax.fori_loop(0, n_chunk, mlp, 0)
        out_copy(n_chunk - 2, (n_chunk - 2) % 2).wait()
        out_copy(n_chunk - 1, (n_chunk - 1) % 2).wait()

    pl.run_scoped(
        mixer,
        pltpu.VMEM((2, RB, D), out_hbm.dtype),
    )


@functools.partial(jax.jit, static_argnames=("A_seg_len",))
def pallas_adaLN_cond__memory_aug_recurrent_mem_tr__mixer_s_mlp__prompt_kernel(
    A_x, A_mem0, A_Wq, A_Wk, A_Wv, A_Wo, A_seg_len,
    B_x, B_w1, B_w2, B_w3, B_w4, c, w_mod,
):
    del B_x
    B, S, D = A_x.shape
    _, H, Dh = A_Wq.shape
    M = A_mem0.shape[1]
    F = B_w3.shape[1]
    seg = int(A_seg_len)
    RB = ROWS
    assert B == 1 and Dh == LANES and S % RB == 0 and RB % seg == 0

    hbm = pl.BlockSpec(memory_space=pl.ANY)
    vmem = pl.BlockSpec(memory_space=pltpu.VMEM)
    dma = pltpu.SemaphoreType.DMA

    out = pl.pallas_call(
        functools.partial(_kernel, S=S, D=D, H=H, Dh=Dh, M=M, seg=seg, F=F, RB=RB),
        out_shape=jax.ShapeDtypeStruct((S, D), A_x.dtype),
        in_specs=[hbm, vmem, hbm, hbm, hbm, hbm, hbm, hbm, hbm, hbm, vmem, hbm],
        out_specs=hbm,
        scratch_shapes=[
            pltpu.VMEM((S, D), A_x.dtype),
            pltpu.VMEM((S, D), F32),
            pltpu.VMEM((S + 2 * SUB, D), F32),
            pltpu.VMEM((6, SUB, D), F32),
            pltpu.VMEM((D, D), BF16),
            pltpu.VMEM((D, F), BF16),
            pltpu.VMEM((F, D), BF16),
            dma((2,)), dma((3,)), dma((D // LANES,)), dma((D // LANES,)),
            dma((4,)), dma((3,)), dma((2,)),
        ],
        compiler_params=pltpu.CompilerParams(vmem_limit_bytes=124 * 1024 * 1024),
    )(
        A_x.reshape(S, D), A_mem0.reshape(M, D), A_Wq, A_Wk, A_Wv,
        A_Wo.reshape(H * Dh, D), B_w1, B_w2, B_w3, B_w4, c, w_mod,
    )
    return out.reshape(B, S, D)
```

```python
import functools

import jax
import jax.numpy as jnp
from jax import lax
import jax.experimental.pallas as pl
import jax.experimental.pallas.tpu as pltpu

F32 = jnp.float32
BF16 = jnp.bfloat16
U32 = jnp.uint32
LANES = 128
SUB = 8
HEAD_TILE = 8
LAG_S = 1
LAG_PV = 4
LAG_V = 2
OUT_T0 = 30
MIX_T = 31
N_PART = 8
N_SPLIT = 2
ROWS = 256
RT = 16
EARLY = 3
BS = 1
RT_FIRST = 0
EPS = 1e-5

_NN = (((1,), (0,)), ((), ()))
_NT = (((1,), (1,)), ((), ()))


def _mm(a, b, dims=_NN):
    return lax.dot_general(a, b, dims, preferred_element_type=F32)


def _bf(w):
    return pltpu.bitcast(w, BF16)


def _layernorm(x):
    m = jnp.mean(x, axis=-1, keepdims=True)
    d = x - m
    v = jnp.mean(d * d, axis=-1, keepdims=True)
    return d * lax.rsqrt(v + EPS)


def _gelu(x):
    k = 0.7978845608028654
    return (0.5 * x) * (1.0 + jnp.tanh(k * (x + 0.044715 * (x * x * x))))


def _lhs7(a11, a12, a21, a22):
    return (a11 + a22, a21 + a22, a11, a22, a11 + a12, a21 - a11, a12 - a22)


def _rhs7(b11, b12, b21, b22):
    f11, f12, f21, f22 = (b.astype(F32) for b in (b11, b12, b21, b22))
    return ((f11 + f22).astype(BF16), b11, (f12 - f22).astype(BF16), (f21 - f11).astype(BF16),
            b22, (f11 + f12).astype(BF16), (f21 + f22).astype(BF16))


def _out4(m1, m2, m3, m4, m5, m6, m7):
    return m1 + m4 - m5 + m7, m3 + m5, m2 + m4, m1 - m2 + m3 + m6


def _kernel(
    x_hbm, mem0_ref, wq_hbm, wk_hbm, wv_hbm, wo_hbm,
    w1_hbm, w2_hbm, w3_hbm, w4_hbm, c_ref, wmod_hbm,
    out_hbm,
    x_s, hx, u_s, mod_s, w2_s, w3_s, w4_s,
    sem_x, sem_stage, sem_wo, sem_w1, sem_mod, sem_b, sem_out,
    *, S, D, H, Dh, M, seg, F, RB,
):
    n_seg = S // seg
    L = M + seg
    n_col = D // LANES
    scale = Dh ** (-0.5)
    ride = seg - M
    ahead = S - n_seg * ride
    ring = ahead + seg
    n_ht = H // HEAD_TILE

    b_copies = [
        pltpu.make_async_copy(src, dst, sem_b.at[i])
        for i, (src, dst) in enumerate(
            ((w2_hbm, w2_s), (w3_hbm, w3_s), (w4_hbm, w4_s)))
    ]

    PAD = SUB
    u_s[:PAD, :] = jnp.zeros((PAD, D), F32)
    u_s[PAD + S:, :] = jnp.zeros((PAD, D), F32)

    def cond(xa):
        return _layernorm(xa) * (1.0 + mod_s[4, 0:1, :]) + mod_s[3, 0:1, :]

    def attention(w_s, wo_s, w1_s, qkv_r, stage, wmod_s, hc_s, *o_s):
        w_hbm = (wq_hbm, wk_hbm, wv_hbm)
        n_w = 3 * n_ht

        def slot(m, h):
            return (3 * (h // HEAD_TILE) + m) * HEAD_TILE + h % HEAD_TILE

        def mod_copy(j, b):
            return pltpu.make_async_copy(
                wmod_hbm.at[:, pl.ds(j * D, D)], wmod_s.at[b], sem_mod.at[b])

        x_head = pltpu.make_async_copy(
            x_hbm.at[pl.ds(0, ahead)], x_s.at[pl.ds(0, ahead)], sem_x.at[0])
        x_tail = pltpu.make_async_copy(
            x_hbm.at[pl.ds(ahead, S - ahead)], x_s.at[pl.ds(ahead, S - ahead)], sem_x.at[1])

        def stage_copy(m, t):
            heads = pl.ds(pl.multiple_of(t * HEAD_TILE, HEAD_TILE), HEAD_TILE)
            return pltpu.make_async_copy(
                w_hbm[m].at[:, heads, :], stage.at[m], sem_stage.at[m])

        def wo_copy(j):
            cols = pl.ds(pl.multiple_of(j * LANES, LANES), LANES)
            return (pltpu.make_async_copy(wo_hbm.at[:, cols], wo_s.at[j], sem_wo.at[j]),
                    pltpu.make_async_copy(w1_hbm.at[:, cols], w1_s.at[j], sem_w1.at[j]))

        stage_copy(0, 0).start()
        mod_copy(0, 0).start()
        mod_copy(1, 1).start()
        x_head.start()

        cv = c_ref[...].astype(F32)
        silu_c = jnp.broadcast_to(cv * (1.0 / (1.0 + jnp.exp(-cv))), (SUB, D))

        def make_mod(j, b):
            mod_copy(j, b).wait()
            mod_s[j] = _mm(silu_c, wmod_s[b])

        def retile(i, pieces=range(D // RT)):
            src = lax.rem(i, 3)
            for r in pieces:
                blk = jnp.transpose(stage[src, r * RT:(r + 1) * RT, :, :], (1, 0, 2))
                for hh in range(HEAD_TILE):
                    w_s[i * HEAD_TILE + hh, r * RT // 2:(r + 1) * RT // 2, :] = (
                        pltpu.bitcast(blk[hh], U32))

        def modulate(start, n):
            rows = pl.ds(pl.multiple_of(start, SUB), n)
            return (_layernorm(x_s[rows, :].astype(F32))
                    * (1.0 + mod_s[1, 0:1, :]) + mod_s[0, 0:1, :])

        stage_copy(0, 0).wait()
        stage_copy(1, 0).start()
        retile(0)
        make_mod(0, 0)
        make_mod(1, 1)
        x_head.wait()
        stage_copy(2, 0).start()

        def head_rows(i, carry):
            hx[pl.ds(pl.multiple_of(i * 64, 64), 64), :] = modulate(i * 64, 64)
            return carry

        lax.fori_loop(0, ahead // 64, head_rows, 0, unroll=2)

        def bulk(i, carry):
            nxt = jnp.minimum(i + 1, n_w - 1)
            for m in range(3):
                @pl.when((i + 3 < n_w) & (lax.rem(i, 3) == m))
                def _():
                    stage_copy(m, i // 3 + 1).start()

                @pl.when((i + 1 < n_w) & (lax.rem(i + 1, 3) == m))
                def _():
                    stage_copy(m, (i + 1) // 3).wait()

            @pl.when(i < n_col)
            def _():
                for cp in wo_copy(i):
                    cp.start()

            @pl.when(i == n_col + 1)
            def _():
                x_tail.start()

            for j in range(4):
                @pl.when(i == n_col - 1 + j)
                def _():
                    mod_copy(2 + j, j).start()

            pc, rs = D // RT // HEAD_TILE // BS, ahead // BS
            for hh in range(HEAD_TILE):
                j = i * HEAD_TILE + hh
                for a in range(BS):
                    p0 = (hh * BS + a) * pc
                    if RT_FIRST:
                        retile(nxt, range(p0, p0 + pc))
                    qkv_r[j, a * rs:(a + 1) * rs, :] = _mm(hx[a * rs:(a + 1) * rs, :], _bf(w_s[j]))
                    if not RT_FIRST:
                        retile(nxt, range(p0, p0 + pc))
            return carry

        lax.fori_loop(0, n_w, bulk, 0)

        for j in range(4):
            make_mod(2 + j, j)
        for cp in b_copies:
            cp.start()
        for j in range(n_col):
            for cp in wo_copy(j):
                cp.wait()

        hc_s[:M, :] = mem0_ref[...].astype(F32)
        x_tail.wait()
        hc_s[M:, :] = modulate(ahead, ride)

        row = lax.broadcasted_iota(jnp.int32, (L, L), 0)
        col = lax.broadcasted_iota(jnp.int32, (L, L), 1)
        mask = (row < M) | (row >= col)
        hpp = H // N_PART
        part = hpp * Dh

        def mix_in(s):
            start = pl.multiple_of(s * seg, seg)
            z = _layernorm(cond(hx[pl.ds(start, seg), :]))
            for j in range(n_col):
                u_s[pl.ds(start + PAD, seg), j * LANES:(j + 1) * LANES] = _gelu(_mm(z, w1_s[j]))

        def step(s, carry):
            rd = pl.ds(pl.multiple_of(lax.rem(s * seg, ring), SUB), seg)
            wr = [pl.ds(pl.multiple_of(lax.rem(ahead + s * ride + j * SUB, ring), SUB), SUB)
                  for j in range(ride // SUB)]
            qkv, ev = {}, {}
            acc = [None] * n_col

            def project(p):
                ks = slice(p * part, (p + 1) * part)
                for j in range(n_col):
                    r = _mm(o_s[p][...], wo_s[j, ks, :])
                    acc[j] = r if acc[j] is None else acc[j] + r

            def project_in(m, h):
                r = _mm(hc_s[...], _bf(w_s[slot(m, h)]))
                for j, rows in enumerate(wr):
                    qkv_r[slot(m, h), rows, :] = r[M + j * SUB:M + (j + 1) * SUB]
                qkv[m, h] = r[:M]

            def gather(m, h):
                return jnp.concatenate([qkv.pop((m, h)), qkv_r[slot(m, h), rd, :]], axis=0)

            n_out = 0
            for t in range(H + LAG_PV):
                hs, hp = t - LAG_S, t - LAG_PV
                if 0 <= hs < H:
                    q, k = gather(0, hs), gather(1, hs).astype(BF16)
                if 0 <= hp < H:
                    v = gather(2, hp).astype(BF16)
                if t < H:
                    project_in(0, t)
                    project_in(1, t)
                if 0 <= t - LAG_V < H:
                    project_in(2, t - LAG_V)
                if t >= OUT_T0 and n_out < N_PART and (n_out + 1) * hpp <= hp:
                    project(n_out)
                    n_out += 1
                if t == MIX_T:
                    mix_in(jnp.maximum(s - 1, 0))
                if 0 <= hs < H:
                    sc = jnp.where(mask, _mm(q, k, _NT) * scale, -1000000000.0)
                    e = jnp.exp(sc - jnp.max(sc, axis=-1, keepdims=True))
                    ev[hs] = e / jnp.sum(e, axis=-1, keepdims=True)
                if 0 <= hp < H:
                    o_s[hp // hpp][:, (hp % hpp) * Dh:(hp % hpp + 1) * Dh] = _mm(ev.pop(hp), v)
            for p in range(n_out, N_PART):
                project(p)
            nxt = jnp.minimum(ahead + (s + 1) * ride, S - ride)
            hc_s[M:, :] = modulate(nxt, ride)
            rows = pl.ds(pl.multiple_of(s * seg, seg), seg)
            for j in range(n_col):
                cols = slice(j * LANES, (j + 1) * LANES)
                hc_s[:M, cols] = acc[j][:M]
                hx[rows, cols] = x_s[rows, cols].astype(F32) + mod_s[2, 0:1, cols] * acc[j][M:]
            return carry

        lax.fori_loop(0, n_seg, step, 0)
        mix_in(n_seg - 1)

    pl.run_scoped(
        attention,
        pltpu.VMEM((3 * H, D // 2, Dh), U32),
        pltpu.VMEM((n_col, H * Dh, LANES), BF16),
        pltpu.VMEM((n_col, D, LANES), BF16),
        pltpu.VMEM((3 * H, ring, Dh), F32),
        pltpu.VMEM((3, D, HEAD_TILE, Dh), BF16),
        pltpu.VMEM((4, D, D), BF16),
        pltpu.VMEM((seg, D), F32),
        *[pltpu.VMEM((L, H * Dh // N_PART), F32)] * N_PART,
    )

    def mixer(w3_7, w4_7, a_s, t_s, out_s):
        hd, hf = D // 2, F // 2
        n_chunk = S // RB
        for cp in b_copies:
            cp.wait()

        def out_copy(i, slot):
            return pltpu.make_async_copy(
                out_s.at[slot], out_hbm.at[pl.ds(pl.multiple_of(i * RB, RB), RB), :],
                sem_out.at[slot])

        cq = D // 4

        def mlp(i, carry, first=False):
            slot = i % 2

            if not first:
                @pl.when(i >= 2)
                def _():
                    out_copy(i - 2, slot).wait()

            rs = RB // N_SPLIT
            x1, t = [], []
            for a in range(N_SPLIT):
                start = pl.multiple_of(i * RB + a * rs, rs)
                parts = []
                for g, off in enumerate((-1, 1, -2, 2)):
                    ug = u_s[pl.ds(start, rs + 2 * PAD), g * cq:(g + 1) * cq]
                    parts.append(ug[PAD + off:PAD + off + rs])
                x1.append(cond(hx[pl.ds(start, rs), :])
                          + _mm(jnp.concatenate(parts, axis=1), w2_s[...]))
            def weights(w, w7, j):
                if not first:
                    return [_bf(w7[j, p]) for p in range(7)]
                hk, hn = w.shape[0] // 2, w.shape[1] // 2
                lo, hi = slice(j * LANES, (j + 1) * LANES), slice(hn + j * LANES, hn + (j + 1) * LANES)
                rhs = _rhs7(w[:hk, lo], w[:hk, hi], w[hk:, lo], w[hk:, hi])
                for p in range(7):
                    w7[j, p] = pltpu.bitcast(rhs[p], U32)
                return rhs

            z = [_layernorm(v) for v in x1]
            for p, v in enumerate(_lhs7(z[0][:, :hd], z[0][:, hd:], z[1][:, :hd], z[1][:, hd:])):
                a_s[p] = v
            rhs = {j: weights(w3_s, w3_7, j) for j in range(EARLY)}
            early = {(j, p): _mm(a_s[p], rhs[j][p]) for j in range(EARLY) for p in (2, 4)}
            for j in range(hf // LANES):
                r7 = rhs[j] if j in rhs else weights(w3_s, w3_7, j)
                cs = _out4(*[early[j, p] if (j, p) in early else _mm(a_s[p], r7[p])
                             for p in range(7)])
                for p, v in enumerate(_lhs7(*[_gelu(v) for v in cs])):
                    t_s[p, :, j * LANES:(j + 1) * LANES] = v
            for j in range(hd // LANES):
                lo, hi = slice(j * LANES, (j + 1) * LANES), slice(hd + j * LANES, hd + (j + 1) * LANES)
                r7 = weights(w4_s, w4_7, j)
                cs = _out4(*[_mm(t_s[p], r7[p]) for p in range(7)])
                for v, a, cols in zip(cs, (0, 0, 1, 1), (lo, hi, lo, hi)):
                    start = pl.multiple_of(i * RB + a * rs, rs)
                    out_s[slot, a * rs:(a + 1) * rs, cols] = (
                        hx[pl.ds(start, rs), cols]
                        + mod_s[5, 0:1, cols] * (x1[a][:, cols] + v)).astype(out_s.dtype)
            out_copy(i, slot).start()
            return carry

        mlp(0, 0, first=True)
        lax.fori_loop(1, n_chunk, mlp, 0)
        out_copy(n_chunk - 2, (n_chunk - 2) % 2).wait()
        out_copy(n_chunk - 1, (n_chunk - 1) % 2).wait()

    pl.run_scoped(
        mixer,
        pltpu.VMEM((F // 2 // LANES, 7, D // 4, LANES), U32),
        pltpu.VMEM((D // 2 // LANES, 7, F // 4, LANES), U32),
        pltpu.VMEM((7, RB // 2, D // 2), F32),
        pltpu.VMEM((7, RB // 2, F // 2), F32),
        pltpu.VMEM((2, RB, D), out_hbm.dtype),
    )


@functools.partial(jax.jit, static_argnames=("A_seg_len",))
def pallas_adaLN_cond__memory_aug_recurrent_mem_tr__mixer_s_mlp__prompt_kernel(
    A_x, A_mem0, A_Wq, A_Wk, A_Wv, A_Wo, A_seg_len,
    B_x, B_w1, B_w2, B_w3, B_w4, c, w_mod,
):
    del B_x
    B, S, D = A_x.shape
    _, H, Dh = A_Wq.shape
    M = A_mem0.shape[1]
    F = B_w3.shape[1]
    seg = int(A_seg_len)
    RB = ROWS
    assert B == 1 and Dh == LANES and S % RB == 0 and RB % seg == 0

    hbm = pl.BlockSpec(memory_space=pl.ANY)
    vmem = pl.BlockSpec(memory_space=pltpu.VMEM)
    dma = pltpu.SemaphoreType.DMA

    out = pl.pallas_call(
        functools.partial(_kernel, S=S, D=D, H=H, Dh=Dh, M=M, seg=seg, F=F, RB=RB),
        out_shape=jax.ShapeDtypeStruct((S, D), A_x.dtype),
        in_specs=[hbm, vmem, hbm, hbm, hbm, hbm, hbm, hbm, hbm, hbm, vmem, hbm],
        out_specs=hbm,
        scratch_shapes=[
            pltpu.VMEM((S, D), A_x.dtype),
            pltpu.VMEM((S, D), F32),
            pltpu.VMEM((S + 2 * SUB, D), F32),
            pltpu.VMEM((6, SUB, D), F32),
            pltpu.VMEM((D, D), BF16),
            pltpu.VMEM((D, F), BF16),
            pltpu.VMEM((F, D), BF16),
            dma((2,)), dma((3,)), dma((D // LANES,)), dma((D // LANES,)),
            dma((4,)), dma((3,)), dma((2,)),
        ],
        compiler_params=pltpu.CompilerParams(vmem_limit_bytes=124 * 1024 * 1024),
    )(
        A_x.reshape(S, D), A_mem0.reshape(M, D), A_Wq, A_Wk, A_Wv,
        A_Wo.reshape(H * Dh, D), B_w1, B_w2, B_w3, B_w4, c, w_mod,
    )
    return out.reshape(B, S, D)
```

```python
import functools

import jax
import jax.numpy as jnp
from jax import lax
import jax.experimental.pallas as pl
import jax.experimental.pallas.tpu as pltpu

F32 = jnp.float32
BF16 = jnp.bfloat16
U32 = jnp.uint32
LANES = 128
SUB = 8
HEAD_TILE = 8
LAG_S = 1
LAG_PV = 3
LAG_V = 1
OUT_T0 = 31
MIX_T = 34
N_PART = 8
N_SPLIT = 2
ROWS = 256
RT = 16
EPS = 1e-5

_NN = (((1,), (0,)), ((), ()))
_NT = (((1,), (1,)), ((), ()))


def _mm(a, b, dims=_NN):
    return lax.dot_general(a, b, dims, preferred_element_type=F32)


def _bf(w):
    return pltpu.bitcast(w, BF16)


def _layernorm(x):
    m = jnp.mean(x, axis=-1, keepdims=True)
    d = x - m
    v = jnp.mean(d * d, axis=-1, keepdims=True)
    return d * lax.rsqrt(v + EPS)


def _gelu(x):
    k = 0.7978845608028654
    return (0.5 * x) * (1.0 + jnp.tanh(k * (x + 0.044715 * (x * x * x))))


def _kernel(
    x_hbm, mem0_ref, wq_hbm, wk_hbm, wv_hbm, wo_hbm,
    w1_hbm, w2_hbm, w3_hbm, w4_hbm, c_ref, wmod_hbm,
    out_hbm,
    x_s, hx, u_s, mod_s, w2_s, w3_s, w4_s,
    sem_x, sem_stage, sem_wo, sem_w1, sem_mod, sem_b, sem_out,
    *, S, D, H, Dh, M, seg, F, RB,
):
    n_seg = S // seg
    L = M + seg
    n_col = D // LANES
    scale = Dh ** (-0.5)
    ride = seg - M
    ahead = S - n_seg * ride
    ring = ahead + seg
    n_ht = H // HEAD_TILE

    b_copies = [
        pltpu.make_async_copy(src, dst, sem_b.at[i])
        for i, (src, dst) in enumerate(
            ((w2_hbm, w2_s), (w3_hbm, w3_s), (w4_hbm, w4_s)))
    ]

    PAD = SUB
    u_s[:PAD, :] = jnp.zeros((PAD, D), F32)
    u_s[PAD + S:, :] = jnp.zeros((PAD, D), F32)

    def cond(xa):
        return _layernorm(xa) * (1.0 + mod_s[4, 0:1, :]) + mod_s[3, 0:1, :]

    def attention(w_s, wo_s, w1_s, qkv_r, stage, wmod_s, hc_s, *o_s):
        w_hbm = (wq_hbm, wk_hbm, wv_hbm)
        n_w = 3 * n_ht

        def slot(m, h):
            return (3 * (h // HEAD_TILE) + m) * HEAD_TILE + h % HEAD_TILE

        def mod_copy(j, b):
            return pltpu.make_async_copy(
                wmod_hbm.at[:, pl.ds(j * D, D)], wmod_s.at[b], sem_mod.at[b])

        x_head = pltpu.make_async_copy(
            x_hbm.at[pl.ds(0, ahead)], x_s.at[pl.ds(0, ahead)], sem_x.at[0])
        x_tail = pltpu.make_async_copy(
            x_hbm.at[pl.ds(ahead, S - ahead)], x_s.at[pl.ds(ahead, S - ahead)], sem_x.at[1])

        def stage_copy(m, t):
            heads = pl.ds(pl.multiple_of(t * HEAD_TILE, HEAD_TILE), HEAD_TILE)
            return pltpu.make_async_copy(
                w_hbm[m].at[:, heads, :], stage.at[m], sem_stage.at[m])

        def wo_copy(j):
            cols = pl.ds(pl.multiple_of(j * LANES, LANES), LANES)
            return (pltpu.make_async_copy(wo_hbm.at[:, cols], wo_s.at[j], sem_wo.at[j]),
                    pltpu.make_async_copy(w1_hbm.at[:, cols], w1_s.at[j], sem_w1.at[j]))

        stage_copy(0, 0).start()
        mod_copy(0, 0).start()
        mod_copy(1, 1).start()
        x_head.start()

        cv = c_ref[...].astype(F32)
        silu_c = jnp.broadcast_to(cv * (1.0 / (1.0 + jnp.exp(-cv))), (SUB, D))

        def make_mod(j, b):
            mod_copy(j, b).wait()
            mod_s[j] = _mm(silu_c, wmod_s[b])

        def retile(i, pieces=range(D // RT)):
            src = lax.rem(i, 3)
            for r in pieces:
                blk = jnp.transpose(stage[src, r * RT:(r + 1) * RT, :, :], (1, 0, 2))
                for hh in range(HEAD_TILE):
                    w_s[i * HEAD_TILE + hh, r * RT // 2:(r + 1) * RT // 2, :] = (
                        pltpu.bitcast(blk[hh], U32))

        def modulate(start, n):
            rows = pl.ds(pl.multiple_of(start, SUB), n)
            return (_layernorm(x_s[rows, :].astype(F32))
                    * (1.0 + mod_s[1, 0:1, :]) + mod_s[0, 0:1, :])

        stage_copy(0, 0).wait()
        stage_copy(1, 0).start()
        retile(0)
        make_mod(0, 0)
        make_mod(1, 1)
        x_head.wait()
        stage_copy(2, 0).start()

        def head_rows(i, carry):
            hx[pl.ds(pl.multiple_of(i * 64, 64), 64), :] = modulate(i * 64, 64)
            return carry

        lax.fori_loop(0, ahead // 64, head_rows, 0, unroll=2)

        def bulk(i, carry):
            nxt = jnp.minimum(i + 1, n_w - 1)
            for m in range(3):
                @pl.when((i + 3 < n_w) & (lax.rem(i, 3) == m))
                def _():
                    stage_copy(m, i // 3 + 1).start()

                @pl.when((i + 1 < n_w) & (lax.rem(i + 1, 3) == m))
                def _():
                    stage_copy(m, (i + 1) // 3).wait()

            @pl.when(i < n_col)
            def _():
                for cp in wo_copy(i):
                    cp.start()

            @pl.when(i == n_col + 1)
            def _():
                x_tail.start()

            for j in range(4):
                @pl.when(i == n_col - 1 + j)
                def _():
                    mod_copy(2 + j, j).start()

            pc = D // RT // HEAD_TILE
            for hh in range(HEAD_TILE):
                j = i * HEAD_TILE + hh
                qkv_r[j, :ahead, :] = _mm(hx[:ahead, :], _bf(w_s[j]))
                retile(nxt, range(hh * pc, (hh + 1) * pc))
            return carry

        lax.fori_loop(0, n_w, bulk, 0)

        for j in range(4):
            make_mod(2 + j, j)
        for cp in b_copies:
            cp.start()
        for j in range(n_col):
            for cp in wo_copy(j):
                cp.wait()

        hc_s[:M, :] = mem0_ref[...].astype(F32)
        x_tail.wait()
        hc_s[M:, :] = modulate(ahead, ride)

        row = lax.broadcasted_iota(jnp.int32, (L, L), 0)
        col = lax.broadcasted_iota(jnp.int32, (L, L), 1)
        mask = (row < M) | (row >= col)
        hpp = H // N_PART
        part = hpp * Dh

        def mix_in(s):
            start = pl.multiple_of(s * seg, seg)
            z = _layernorm(cond(hx[pl.ds(start, seg), :]))
            for j in range(n_col):
                u_s[pl.ds(start + PAD, seg), j * LANES:(j + 1) * LANES] = _gelu(_mm(z, w1_s[j]))

        def step(s, carry):
            rd = pl.ds(pl.multiple_of(lax.rem(s * seg, ring), SUB), seg)
            wr = [pl.ds(pl.multiple_of(lax.rem(ahead + s * ride + j * SUB, ring), SUB), SUB)
                  for j in range(ride // SUB)]
            qkv, ev = {}, {}
            acc = [None] * n_col

            def project(p):
                ks = slice(p * part, (p + 1) * part)
                for j in range(n_col):
                    r = _mm(o_s[p][...], wo_s[j, ks, :])
                    acc[j] = r if acc[j] is None else acc[j] + r

            def project_in(m, h):
                r = _mm(hc_s[...], _bf(w_s[slot(m, h)]))
                for j, rows in enumerate(wr):
                    qkv_r[slot(m, h), rows, :] = r[M + j * SUB:M + (j + 1) * SUB]
                qkv[m, h] = r[:M]

            def gather(m, h):
                return jnp.concatenate([qkv.pop((m, h)), qkv_r[slot(m, h), rd, :]], axis=0)

            n_out = 0
            for t in range(H + LAG_PV):
                hs, hp = t - LAG_S, t - LAG_PV
                if 0 <= hs < H:
                    q, k = gather(0, hs), gather(1, hs).astype(BF16)
                if 0 <= hp < H:
                    v = gather(2, hp).astype(BF16)
                if t < H:
                    project_in(0, t)
                    project_in(1, t)
                if 0 <= t - LAG_V < H:
                    project_in(2, t - LAG_V)
                if t >= OUT_T0 and n_out < N_PART and (n_out + 1) * hpp <= hp:
                    project(n_out)
                    n_out += 1
                if t == MIX_T:
                    mix_in(jnp.maximum(s - 1, 0))
                if 0 <= hs < H:
                    sc = jnp.where(mask, _mm(q, k, _NT) * scale, -1000000000.0)
                    e = jnp.exp(sc - jnp.max(sc, axis=-1, keepdims=True))
                    ev[hs] = e / jnp.sum(e, axis=-1, keepdims=True)
                if 0 <= hp < H:
                    o_s[hp // hpp][:, (hp % hpp) * Dh:(hp % hpp + 1) * Dh] = _mm(ev.pop(hp), v)
            for p in range(n_out, N_PART):
                project(p)
            nxt = jnp.minimum(ahead + (s + 1) * ride, S - ride)
            hc_s[M:, :] = modulate(nxt, ride)
            rows = pl.ds(pl.multiple_of(s * seg, seg), seg)
            for j in range(n_col):
                cols = slice(j * LANES, (j + 1) * LANES)
                hc_s[:M, cols] = acc[j][:M]
                hx[rows, cols] = x_s[rows, cols].astype(F32) + mod_s[2, 0:1, cols] * acc[j][M:]
            return carry

        lax.fori_loop(0, n_seg, step, 0)
        mix_in(n_seg - 1)

    pl.run_scoped(
        attention,
        pltpu.VMEM((3 * H, D // 2, Dh), U32),
        pltpu.VMEM((n_col, H * Dh, LANES), BF16),
        pltpu.VMEM((n_col, D, LANES), BF16),
        pltpu.VMEM((3 * H, ring, Dh), F32),
        pltpu.VMEM((3, D, HEAD_TILE, Dh), BF16),
        pltpu.VMEM((4, D, D), BF16),
        pltpu.VMEM((seg, D), F32),
        *[pltpu.VMEM((L, H * Dh // N_PART), F32)] * N_PART,
    )

    def mixer(out_s):
        n_chunk = S // RB
        for cp in b_copies:
            cp.wait()

        def out_copy(i, slot):
            return pltpu.make_async_copy(
                out_s.at[slot], out_hbm.at[pl.ds(pl.multiple_of(i * RB, RB), RB), :],
                sem_out.at[slot])

        cq = D // 4

        def mlp(i, carry):
            slot = i % 2

            @pl.when(i >= 2)
            def _():
                out_copy(i - 2, slot).wait()

            rs = RB // N_SPLIT
            x1, t = [], []
            for a in range(N_SPLIT):
                start = pl.multiple_of(i * RB + a * rs, rs)
                parts = []
                for g, off in enumerate((-1, 1, -2, 2)):
                    ug = u_s[pl.ds(start, rs + 2 * PAD), g * cq:(g + 1) * cq]
                    parts.append(ug[PAD + off:PAD + off + rs])
                x1.append(cond(hx[pl.ds(start, rs), :])
                          + _mm(jnp.concatenate(parts, axis=1), w2_s[...]))
            for a in range(N_SPLIT):
                t.append(_gelu(_mm(_layernorm(x1[a]), w3_s[...])))
            for a in range(N_SPLIT):
                start = pl.multiple_of(i * RB + a * rs, rs)
                y = x1[a] + _mm(t[a], w4_s[...])
                out_s[slot, a * rs:(a + 1) * rs, :] = (
                    hx[pl.ds(start, rs), :] + mod_s[5, 0:1, :] * y).astype(out_s.dtype)
            out_copy(i, slot).start()
            return carry

        lax.fori_loop(0, n_chunk, mlp, 0)
        out_copy(n_chunk - 2, (n_chunk - 2) % 2).wait()
        out_copy(n_chunk - 1, (n_chunk - 1) % 2).wait()

    pl.run_scoped(
        mixer,
        pltpu.VMEM((2, RB, D), out_hbm.dtype),
    )


@functools.partial(jax.jit, static_argnames=("A_seg_len",))
def pallas_adaLN_cond__memory_aug_recurrent_mem_tr__mixer_s_mlp__prompt_kernel(
    A_x, A_mem0, A_Wq, A_Wk, A_Wv, A_Wo, A_seg_len,
    B_x, B_w1, B_w2, B_w3, B_w4, c, w_mod,
):
    del B_x
    B, S, D = A_x.shape
    _, H, Dh = A_Wq.shape
    M = A_mem0.shape[1]
    F = B_w3.shape[1]
    seg = int(A_seg_len)
    RB = ROWS
    assert B == 1 and Dh == LANES and S % RB == 0 and RB % seg == 0

    hbm = pl.BlockSpec(memory_space=pl.ANY)
    vmem = pl.BlockSpec(memory_space=pltpu.VMEM)
    dma = pltpu.SemaphoreType.DMA

    out = pl.pallas_call(
        functools.partial(_kernel, S=S, D=D, H=H, Dh=Dh, M=M, seg=seg, F=F, RB=RB),
        out_shape=jax.ShapeDtypeStruct((S, D), A_x.dtype),
        in_specs=[hbm, vmem, hbm, hbm, hbm, hbm, hbm, hbm, hbm, hbm, vmem, hbm],
        out_specs=hbm,
        scratch_shapes=[
            pltpu.VMEM((S, D), A_x.dtype),
            pltpu.VMEM((S, D), F32),
            pltpu.VMEM((S + 2 * SUB, D), F32),
            pltpu.VMEM((6, SUB, D), F32),
            pltpu.VMEM((D, D), BF16),
            pltpu.VMEM((D, F), BF16),
            pltpu.VMEM((F, D), BF16),
            dma((2,)), dma((3,)), dma((D // LANES,)), dma((D // LANES,)),
            dma((4,)), dma((3,)), dma((2,)),
        ],
        compiler_params=pltpu.CompilerParams(vmem_limit_bytes=124 * 1024 * 1024),
    )(
        A_x.reshape(S, D), A_mem0.reshape(M, D), A_Wq, A_Wk, A_Wv,
        A_Wo.reshape(H * Dh, D), B_w1, B_w2, B_w3, B_w4, c, w_mod,
    )
    return out.reshape(B, S, D)
```

```python
import functools

import jax
import jax.numpy as jnp
import numpy as np
from jax import lax
import jax.experimental.pallas as pl
import jax.experimental.pallas.tpu as pltpu

F32 = jnp.float32
BF16 = jnp.bfloat16
U32 = jnp.uint32
LANES = 128
SUB = 8
HEAD_TILE = 8
LAG_S = 1
LAG_PV = 3
LAG_V = 1
OUT_T0 = 31
MIX_T = 34
N_PART = 8
N_SPLIT = 2
ROWS = 256
RT = 16
SKIPB = 0
EPS = 1e-5

_NN = (((1,), (0,)), ((), ()))
_NT = (((1,), (1,)), ((), ()))


def _mm(a, b, dims=_NN):
    return lax.dot_general(a, b, dims, preferred_element_type=F32)


def _bf(w):
    return pltpu.bitcast(w, BF16)


def _layernorm(x):
    m = jnp.mean(x, axis=-1, keepdims=True)
    d = x - m
    v = jnp.mean(d * d, axis=-1, keepdims=True)
    return d * lax.rsqrt(v + EPS)


def _gelu(x):
    k = 0.7978845608028654
    return (0.5 * x) * (1.0 + jnp.tanh(k * (x + 0.044715 * (x * x * x))))


def _split_heads(row):
    sub = lax.broadcasted_iota(jnp.int32, (SUB, LANES), 0)

    def words(d):
        return jnp.concatenate(
            [pltpu.bitcast(row(d), U32), pltpu.bitcast(row(d + SUB), U32)], axis=0)

    def swap(a, b, k):
        keep = (sub & k) == 0
        return (jnp.where(keep, a, pltpu.roll(b, k, 0)),
                jnp.where(keep, pltpu.roll(a, SUB - k, 0), b))

    pairs = [(words(2 * a), words(2 * a + 1)) for a in range(4)]
    lo = [(e & 0xFFFF) | (o << 16) for e, o in pairs]
    hi = [(e >> 16) | (o & np.uint32(0xFFFF0000)) for e, o in pairs]
    for v in (lo, hi):
        v[0], v[1] = swap(v[0], v[1], 1)
        v[2], v[3] = swap(v[2], v[3], 1)
        v[0], v[2] = swap(v[0], v[2], 2)
        v[1], v[3] = swap(v[1], v[3], 2)
    return [v[p] for p in range(4) for v in (lo, hi)]


def _kernel(
    x_hbm, mem0_ref, wq_hbm, wk_hbm, wv_hbm, wo_hbm,
    w1_hbm, w2_hbm, w3_hbm, w4_hbm, c_ref, wmod_hbm,
    out_hbm,
    x_s, hx, u_s, mod_s, w2_s, w3_s, w4_s,
    sem_x, sem_stage, sem_wo, sem_w1, sem_mod, sem_b, sem_out,
    *, S, D, H, Dh, M, seg, F, RB,
):
    n_seg = S // seg
    L = M + seg
    n_col = D // LANES
    scale = Dh ** (-0.5)
    ride = seg - M
    ahead = S - n_seg * ride
    ring = ahead + seg
    n_ht = H // HEAD_TILE

    b_copies = [
        pltpu.make_async_copy(src, dst, sem_b.at[i])
        for i, (src, dst) in enumerate(
            ((w2_hbm, w2_s), (w3_hbm, w3_s), (w4_hbm, w4_s)))
    ]

    PAD = SUB
    u_s[:PAD, :] = jnp.zeros((PAD, D), F32)
    u_s[PAD + S:, :] = jnp.zeros((PAD, D), F32)

    def cond(xa):
        return _layernorm(xa) * (1.0 + mod_s[4, 0:1, :]) + mod_s[3, 0:1, :]

    def attention(w_s, wo_s, w1_s, qkv_r, stage, wmod_s, hc_s, *o_s):
        w_hbm = (wq_hbm, wk_hbm, wv_hbm)
        n_w = 3 * n_ht

        def slot(m, h):
            return (3 * (h // HEAD_TILE) + m) * HEAD_TILE + h % HEAD_TILE

        def mod_copy(j, b):
            return pltpu.make_async_copy(
                wmod_hbm.at[:, pl.ds(j * D, D)], wmod_s.at[b, :, pl.ds(0, D)], sem_mod.at[b])

        x_head = pltpu.make_async_copy(
            x_hbm.at[pl.ds(0, ahead)], x_s.at[pl.ds(0, ahead)], sem_x.at[0])
        x_tail = pltpu.make_async_copy(
            x_hbm.at[pl.ds(ahead, S - ahead)], x_s.at[pl.ds(ahead, S - ahead)], sem_x.at[1])

        def stage_copy(m, t):
            heads = pl.ds(pl.multiple_of(t * HEAD_TILE, HEAD_TILE), HEAD_TILE)
            return pltpu.make_async_copy(
                w_hbm[m].at[:, heads, :], stage.at[m], sem_stage.at[m])

        def wo_copy(j):
            cols = pl.ds(pl.multiple_of(j * LANES, LANES), LANES)
            return (pltpu.make_async_copy(wo_hbm.at[:, cols], wo_s.at[j], sem_wo.at[j]),
                    pltpu.make_async_copy(w1_hbm.at[:, cols], w1_s.at[j], sem_w1.at[j]))

        x_head.start()
        stage_copy(0, 0).start()
        mod_copy(0, 0).start()

        cv = c_ref[...].astype(F32)
        silu_c = jnp.broadcast_to(cv * (1.0 / (1.0 + jnp.exp(-cv))), (SUB, D))

        def make_mod(j, b):
            mod_copy(j, b).wait()
            mod_s[j] = _mm(silu_c, wmod_s[b, :, :D])

        def retile(i, pieces=range(D // RT)):
            src = lax.rem(i, 3)
            for r in pieces:
                for hh, w in enumerate(_split_heads(lambda d: stage[src, r * RT + d])):
                    w_s[i * HEAD_TILE + hh, r * SUB:(r + 1) * SUB, :] = w

        def modulate(start, n):
            rows = pl.ds(pl.multiple_of(start, SUB), n)
            return (_layernorm(x_s[rows, :].astype(F32))
                    * (1.0 + mod_s[1, 0:1, :]) + mod_s[0, 0:1, :])

        x_head.wait()
        mod_copy(1, 1).start()

        @pl.loop(0, ahead // 64, unroll=2)
        def _(i):
            rows = pl.ds(pl.multiple_of(i * 64, 64), 64)
            hx[rows, :] = _layernorm(x_s[rows, :].astype(F32))

        stage_copy(0, 0).wait()
        stage_copy(1, 0).start()
        retile(0)
        make_mod(0, 0)
        make_mod(1, 1)
        stage_copy(2, 0).start()
        hx[:ahead, :] = hx[:ahead, :] * (1.0 + mod_s[1, 0:1, :]) + mod_s[0, 0:1, :]

        def bulk(i, carry):
            nxt = jnp.minimum(i + 1, n_w - 1)
            for m in range(3):
                @pl.when((i + 3 < n_w) & (lax.rem(i, 3) == m))
                def _():
                    stage_copy(m, i // 3 + 1).start()

                @pl.when((i + 1 < n_w) & (lax.rem(i + 1, 3) == m))
                def _():
                    stage_copy(m, (i + 1) // 3).wait()

            @pl.when(i < n_col)
            def _():
                for cp in wo_copy(i):
                    cp.start()

            @pl.when(i == n_col + 1)
            def _():
                x_tail.start()

            for j in range(4):
                @pl.when(i == n_col - 1 + j)
                def _():
                    mod_copy(2 + j, j).start()

            cuts = (0, 1, D // RT // 2, D // RT)
            for hh in range(HEAD_TILE):
                j = i * HEAD_TILE + hh
                qkv_r[j, :ahead, :] = _mm(hx[:ahead, :], _bf(w_s[j]))
                if hh + 1 < len(cuts):
                    retile(nxt, range(cuts[hh], cuts[hh + 1]))
            return carry

        lax.fori_loop(0, n_w, bulk, 0)

        for j in range(4):
            make_mod(2 + j, j)
        for cp in b_copies:
            cp.start()
        for j in range(n_col):
            for cp in wo_copy(j):
                cp.wait()

        hc_s[:M, :] = mem0_ref[...].astype(F32)
        x_tail.wait()
        hc_s[M:, :] = modulate(ahead, ride)

        row = lax.broadcasted_iota(jnp.int32, (L, L), 0)
        col = lax.broadcasted_iota(jnp.int32, (L, L), 1)
        mask = (row < M) | (row >= col)
        hpp = H // N_PART
        part = hpp * Dh

        def mix_in(s):
            start = pl.multiple_of(s * seg, seg)
            z = _layernorm(cond(hx[pl.ds(start, seg), :]))
            for j in range(n_col):
                u_s[pl.ds(start + PAD, seg), j * LANES:(j + 1) * LANES] = _gelu(_mm(z, w1_s[j]))

        def step(s, carry):
            rd = pl.ds(pl.multiple_of(lax.rem(s * seg, ring), SUB), seg)
            wr = [pl.ds(pl.multiple_of(lax.rem(ahead + s * ride + j * SUB, ring), SUB), SUB)
                  for j in range(ride // SUB)]
            qkv, ev = {}, {}
            acc = [None] * n_col

            def project(p):
                ks = slice(p * part, (p + 1) * part)
                for j in range(n_col):
                    r = _mm(o_s[p][...], wo_s[j, ks, :])
                    acc[j] = r if acc[j] is None else acc[j] + r

            def project_in(m, h):
                r = _mm(hc_s[...], _bf(w_s[slot(m, h)]))
                for j, rows in enumerate(wr):
                    qkv_r[slot(m, h), rows, :] = r[M + j * SUB:M + (j + 1) * SUB]
                qkv[m, h] = r[:M]

            def gather(m, h):
                return jnp.concatenate([qkv.pop((m, h)), qkv_r[slot(m, h), rd, :]], axis=0)

            n_out = 0
            for t in range(H + LAG_PV):
                hs, hp = t - LAG_S, t - LAG_PV
                if 0 <= hs < H:
                    q, k = gather(0, hs), gather(1, hs).astype(BF16)
                if 0 <= hp < H:
                    v = gather(2, hp).astype(BF16)
                if t < H:
                    project_in(0, t)
                    project_in(1, t)
                if 0 <= t - LAG_V < H:
                    project_in(2, t - LAG_V)
                if t >= OUT_T0 and n_out < N_PART and (n_out + 1) * hpp <= hp:
                    project(n_out)
                    n_out += 1
                if t == MIX_T:
                    mix_in(jnp.maximum(s - 1, 0))
                if 0 <= hs < H:
                    sc = jnp.where(mask, _mm(q, k, _NT) * scale, -1000000000.0)
                    e = jnp.exp(sc - jnp.max(sc, axis=-1, keepdims=True))
                    ev[hs] = e / jnp.sum(e, axis=-1, keepdims=True)
                if 0 <= hp < H:
                    o_s[hp // hpp][:, (hp % hpp) * Dh:(hp % hpp + 1) * Dh] = _mm(ev.pop(hp), v)
            for p in range(n_out, N_PART):
                project(p)
            nxt = jnp.minimum(ahead + (s + 1) * ride, S - ride)
            hc_s[M:, :] = modulate(nxt, ride)
            rows = pl.ds(pl.multiple_of(s * seg, seg), seg)
            for j in range(n_col):
                cols = slice(j * LANES, (j + 1) * LANES)
                hc_s[:M, cols] = acc[j][:M]
                hx[rows, cols] = x_s[rows, cols].astype(F32) + mod_s[2, 0:1, cols] * acc[j][M:]
            return carry

        lax.fori_loop(0, n_seg, step, 0)
        mix_in(n_seg - 1)

    pl.run_scoped(
        attention,
        pltpu.VMEM((3 * H, D // 2, Dh), U32),
        pltpu.VMEM((n_col, H * Dh, LANES), BF16),
        pltpu.VMEM((n_col, D, LANES), BF16),
        pltpu.VMEM((3 * H, ring, Dh), F32),
        pltpu.VMEM((3, D, HEAD_TILE, Dh), BF16),
        pltpu.VMEM((4, D, D + LANES), BF16),
        pltpu.VMEM((seg, D), F32),
        *[pltpu.VMEM((L, H * Dh // N_PART), F32)] * N_PART,
    )

    def mixer(out_s):
        n_chunk = S // RB
        for cp in b_copies:
            cp.wait()

        def out_copy(i, slot):
            return pltpu.make_async_copy(
                out_s.at[slot], out_hbm.at[pl.ds(pl.multiple_of(i * RB, RB), RB), :],
                sem_out.at[slot])

        cq = D // 4

        def mlp(i, carry):
            slot = i % 2

            @pl.when(i >= 2)
            def _():
                out_copy(i - 2, slot).wait()

            rs = RB // N_SPLIT
            x1, t = [], []
            for a in range(N_SPLIT):
                start = pl.multiple_of(i * RB + a * rs, rs)
                parts = []
                for g, off in enumerate((-1, 1, -2, 2)):
                    ug = u_s[pl.ds(start, rs + 2 * PAD), g * cq:(g + 1) * cq]
                    parts.append(ug[PAD + off:PAD + off + rs])
                x1.append(cond(hx[pl.ds(start, rs), :])
                          + _mm(jnp.concatenate(parts, axis=1), w2_s[...]))
            for a in range(N_SPLIT):
                t.append(_gelu(_mm(_layernorm(x1[a]), w3_s[...])))
            for a in range(N_SPLIT):
                start = pl.multiple_of(i * RB + a * rs, rs)
                y = x1[a] + _mm(t[a], w4_s[...])
                out_s[slot, a * rs:(a + 1) * rs, :] = (
                    hx[pl.ds(start, rs), :] + mod_s[5, 0:1, :] * y).astype(out_s.dtype)
            out_copy(i, slot).start()
            return carry

        if SKIPB: return
        lax.fori_loop(0, n_chunk, mlp, 0)
        out_copy(n_chunk - 2, (n_chunk - 2) % 2).wait()
        out_copy(n_chunk - 1, (n_chunk - 1) % 2).wait()

    pl.run_scoped(
        mixer,
        pltpu.VMEM((2, RB, D), out_hbm.dtype),
    )


@functools.partial(jax.jit, static_argnames=("A_seg_len",))
def pallas_adaLN_cond__memory_aug_recurrent_mem_tr__mixer_s_mlp__prompt_kernel(
    A_x, A_mem0, A_Wq, A_Wk, A_Wv, A_Wo, A_seg_len,
    B_x, B_w1, B_w2, B_w3, B_w4, c, w_mod,
):
    del B_x
    B, S, D = A_x.shape
    _, H, Dh = A_Wq.shape
    M = A_mem0.shape[1]
    F = B_w3.shape[1]
    seg = int(A_seg_len)
    RB = ROWS
    assert B == 1 and Dh == LANES and S % RB == 0 and RB % seg == 0

    hbm = pl.BlockSpec(memory_space=pl.ANY)
    vmem = pl.BlockSpec(memory_space=pltpu.VMEM)
    dma = pltpu.SemaphoreType.DMA

    out = pl.pallas_call(
        functools.partial(_kernel, S=S, D=D, H=H, Dh=Dh, M=M, seg=seg, F=F, RB=RB),
        out_shape=jax.ShapeDtypeStruct((S, D), A_x.dtype),
        in_specs=[hbm, vmem, hbm, hbm, hbm, hbm, hbm, hbm, hbm, hbm, vmem, hbm],
        out_specs=hbm,
        scratch_shapes=[
            pltpu.VMEM((S, D), A_x.dtype),
            pltpu.VMEM((S, D), F32),
            pltpu.VMEM((S + 2 * SUB, D), F32),
            pltpu.VMEM((6, SUB, D), F32),
            pltpu.VMEM((D, D), BF16),
            pltpu.VMEM((D, F), BF16),
            pltpu.VMEM((F, D), BF16),
            dma((2,)), dma((3,)), dma((D // LANES,)), dma((D // LANES,)),
            dma((4,)), dma((3,)), dma((2,)),
        ],
        compiler_params=pltpu.CompilerParams(vmem_limit_bytes=124 * 1024 * 1024),
    )(
        A_x.reshape(S, D), A_mem0.reshape(M, D), A_Wq, A_Wk, A_Wv,
        A_Wo.reshape(H * Dh, D), B_w1, B_w2, B_w3, B_w4, c, w_mod,
    )
    return out.reshape(B, S, D)
```

```python
import functools

import jax
import jax.numpy as jnp
import numpy as np
from jax import lax
import jax.experimental.pallas as pl
import jax.experimental.pallas.tpu as pltpu

F32 = jnp.float32
BF16 = jnp.bfloat16
U32 = jnp.uint32
LANES = 128
SUB = 8
HEAD_TILE = 8
PIECE = 16
LAG_V, LAG_S, LAG_PV = 1, 1, 3
N_PART = 8
ROWS = 256
N_SPLIT = 2
EPS = 1e-5

_NN = (((1,), (0,)), ((), ()))
_NT = (((1,), (1,)), ((), ()))


def _mm(a, b, dims=_NN):
    return lax.dot_general(a, b, dims, preferred_element_type=F32)


def _layernorm(x):
    m = jnp.mean(x, axis=-1, keepdims=True)
    d = x - m
    v = jnp.mean(d * d, axis=-1, keepdims=True)
    return d * lax.rsqrt(v + EPS)


def _gelu(x):
    k = 0.7978845608028654
    return (0.5 * x) * (1.0 + jnp.tanh(k * (x + 0.044715 * (x * x * x))))


def _split_heads(row):
    sub = lax.broadcasted_iota(jnp.int32, (SUB, LANES), 0)

    def words(d):
        return jnp.concatenate(
            [pltpu.bitcast(row(d), U32), pltpu.bitcast(row(d + SUB), U32)], axis=0)

    def swap(a, b, k):
        keep = (sub & k) == 0
        return (jnp.where(keep, a, pltpu.roll(b, k, 0)),
                jnp.where(keep, pltpu.roll(a, SUB - k, 0), b))

    pairs = [(words(2 * a), words(2 * a + 1)) for a in range(4)]
    lo = [(e & 0xFFFF) | (o << 16) for e, o in pairs]
    hi = [(e >> 16) | (o & np.uint32(0xFFFF0000)) for e, o in pairs]
    for v in (lo, hi):
        v[0], v[1] = swap(v[0], v[1], 1)
        v[2], v[3] = swap(v[2], v[3], 1)
        v[0], v[2] = swap(v[0], v[2], 2)
        v[1], v[3] = swap(v[1], v[3], 2)
    return [v[p] for p in range(4) for v in (lo, hi)]


def _kernel(
    x_hbm, mem0_ref, wq_hbm, wk_hbm, wv_hbm, wo_hbm,
    w1_hbm, w2_hbm, w3_hbm, w4_hbm, c_ref, wmod_hbm,
    out_hbm,
    x_s, hx, u_s, mod_s, w2_s, w3_s, w4_s,
    sem_x, sem_stage, sem_wo, sem_w1, sem_mod, sem_b, sem_out,
    *, seg,
):
    S, D = x_hbm.shape
    _, H, Dh = wq_hbm.shape
    M = mem0_ref.shape[0]
    n_seg = S // seg
    L = M + seg
    n_col = D // LANES
    n_w = 3 * H // HEAD_TILE
    scale = Dh ** (-0.5)
    ride = seg - M
    ahead = S - n_seg * ride
    ring = ahead + seg
    PAD = SUB
    assert n_col + 3 <= n_w and ahead % 64 == 0 and ring % seg == 0

    def mod(j):
        return mod_s[j, 0:1, :]

    def cond(xa):
        return _layernorm(xa) * (1.0 + mod(4)) + mod(3)

    b_copies = [
        pltpu.make_async_copy(src, dst, sem_b.at[i])
        for i, (src, dst) in enumerate(((w2_hbm, w2_s), (w3_hbm, w3_s), (w4_hbm, w4_s)))
    ]
    u_s[:PAD, :] = jnp.zeros((PAD, D), F32)
    u_s[PAD + S:, :] = jnp.zeros((PAD, D), F32)

    def attention(w_s, wo_s, w1_s, qkv_r, stage, wmod_s, hc_s, *o_s):
        w_hbm = (wq_hbm, wk_hbm, wv_hbm)

        def slot(m, h):
            return (3 * (h // HEAD_TILE) + m) * HEAD_TILE + h % HEAD_TILE

        def weight(j):
            return pltpu.bitcast(w_s[j], BF16)

        def mod_copy(j, b):
            return pltpu.make_async_copy(
                wmod_hbm.at[:, pl.ds(j * D, D)], wmod_s.at[b, :, pl.ds(0, D)], sem_mod.at[b])

        def x_copy(start, n, b):
            return pltpu.make_async_copy(
                x_hbm.at[pl.ds(start, n)], x_s.at[pl.ds(start, n)], sem_x.at[b])

        def stage_copy(m, t):
            heads = pl.ds(pl.multiple_of(t * HEAD_TILE, HEAD_TILE), HEAD_TILE)
            return pltpu.make_async_copy(
                w_hbm[m].at[:, heads, :], stage.at[m], sem_stage.at[m])

        def col_copies(j):
            cols = pl.ds(pl.multiple_of(j * LANES, LANES), LANES)
            return (pltpu.make_async_copy(wo_hbm.at[:, cols], wo_s.at[j], sem_wo.at[j]),
                    pltpu.make_async_copy(w1_hbm.at[:, cols], w1_s.at[j], sem_w1.at[j]))

        x_head, x_tail = x_copy(0, ahead, 0), x_copy(ahead, S - ahead, 1)
        x_head.start()
        stage_copy(0, 0).start()
        mod_copy(0, 0).start()

        cv = c_ref[...].astype(F32)
        silu_c = jnp.broadcast_to(cv * (1.0 / (1.0 + jnp.exp(-cv))), (SUB, D))

        def make_mod(j, b):
            mod_copy(j, b).wait()
            mod_s[j] = _mm(silu_c, wmod_s[b, :, :D])

        def retile(i, pieces):
            src = lax.rem(i, 3)
            for r in pieces:
                for hh, w in enumerate(_split_heads(lambda d: stage[src, r * PIECE + d])):
                    w_s[i * HEAD_TILE + hh, r * SUB:(r + 1) * SUB, :] = w

        x_head.wait()
        mod_copy(1, 1).start()

        @pl.loop(0, ahead // 64, unroll=2)
        def _(i):
            rows = pl.ds(pl.multiple_of(i * 64, 64), 64)
            hx[rows, :] = _layernorm(x_s[rows, :].astype(F32))

        stage_copy(0, 0).wait()
        stage_copy(1, 0).start()
        retile(0, range(D // PIECE))
        make_mod(0, 0)
        make_mod(1, 1)
        stage_copy(2, 0).start()
        hx[:ahead, :] = hx[:ahead, :] * (1.0 + mod(1)) + mod(0)

        def bulk(i, carry):
            nxt = jnp.minimum(i + 1, n_w - 1)
            for m in range(3):
                @pl.when((i + 3 < n_w) & (lax.rem(i, 3) == m))
                def _():
                    stage_copy(m, i // 3 + 1).start()

                @pl.when((i + 1 < n_w) & (lax.rem(i + 1, 3) == m))
                def _():
                    stage_copy(m, (i + 1) // 3).wait()

            @pl.when(i < n_col)
            def _():
                for cp in col_copies(i):
                    cp.start()

            @pl.when(i == n_col + 1)
            def _():
                x_tail.start()

            for j in range(4):
                @pl.when(i == n_col - 1 + j)
                def _():
                    mod_copy(2 + j, j).start()

            cuts = (0, 1, D // PIECE // 2, D // PIECE)
            for hh in range(HEAD_TILE):
                j = i * HEAD_TILE + hh
                qkv_r[j, :ahead, :] = _mm(hx[:ahead, :], weight(j))
                if hh + 1 < len(cuts):
                    retile(nxt, range(cuts[hh], cuts[hh + 1]))
            return carry

        lax.fori_loop(0, n_w, bulk, 0)

        for j in range(4):
            make_mod(2 + j, j)
        for cp in b_copies:
            cp.start()
        for j in range(n_col):
            for cp in col_copies(j):
                cp.wait()

        def riders(start):
            rows = pl.ds(pl.multiple_of(start, SUB), ride)
            return _layernorm(x_s[rows, :].astype(F32)) * (1.0 + mod(1)) + mod(0)

        hc_s[:M, :] = mem0_ref[...].astype(F32)
        x_tail.wait()
        hc_s[M:, :] = riders(ahead)

        row = lax.broadcasted_iota(jnp.int32, (L, L), 0)
        col = lax.broadcasted_iota(jnp.int32, (L, L), 1)
        mask = (row < M) | (row >= col)
        hpp = H // N_PART

        def mix_in(s):
            start = pl.multiple_of(s * seg, seg)
            z = _layernorm(cond(hx[pl.ds(start, seg), :]))
            for j in range(n_col):
                u_s[pl.ds(start + PAD, seg), j * LANES:(j + 1) * LANES] = _gelu(_mm(z, w1_s[j]))

        def step(s, carry):
            rd = pl.ds(pl.multiple_of(lax.rem(s * seg, ring), SUB), seg)
            wr = [pl.ds(pl.multiple_of(lax.rem(ahead + s * ride + j * SUB, ring), SUB), SUB)
                  for j in range(ride // SUB)]
            mem_rows, probs = {}, {}
            acc = [None] * n_col

            def project_in(m, h):
                r = _mm(hc_s[...], weight(slot(m, h)))
                for j, rows in enumerate(wr):
                    qkv_r[slot(m, h), rows, :] = r[M + j * SUB:M + (j + 1) * SUB]
                mem_rows[m, h] = r[:M]

            def gather(m, h):
                return jnp.concatenate(
                    [mem_rows.pop((m, h)), qkv_r[slot(m, h), rd, :]], axis=0)

            def project_out(p):
                ks = slice(p * hpp * Dh, (p + 1) * hpp * Dh)
                for j in range(n_col):
                    r = _mm(o_s[p][...], wo_s[j, ks, :])
                    acc[j] = r if acc[j] is None else acc[j] + r

            n_out = 0
            for t in range(H + LAG_PV):
                hs, hp = t - LAG_S, t - LAG_PV
                if 0 <= hs < H:
                    q, k = gather(0, hs), gather(1, hs).astype(BF16)
                if 0 <= hp < H:
                    v = gather(2, hp).astype(BF16)
                if t < H:
                    project_in(0, t)
                    project_in(1, t)
                if 0 <= t - LAG_V < H:
                    project_in(2, t - LAG_V)
                if t >= H - 1 and (n_out + 1) * hpp <= hp:
                    project_out(n_out)
                    n_out += 1
                if t == H + LAG_PV - 1:
                    mix_in(jnp.maximum(s - 1, 0))
                if 0 <= hs < H:
                    sc = jnp.where(mask, _mm(q, k, _NT) * scale, -1000000000.0)
                    e = jnp.exp(sc - jnp.max(sc, axis=-1, keepdims=True))
                    probs[hs] = e / jnp.sum(e, axis=-1, keepdims=True)
                if 0 <= hp < H:
                    o_s[hp // hpp][:, (hp % hpp) * Dh:(hp % hpp + 1) * Dh] = (
                        _mm(probs.pop(hp), v))
            for p in range(n_out, N_PART):
                project_out(p)
            hc_s[M:, :] = riders(jnp.minimum(ahead + (s + 1) * ride, S - ride))
            rows = pl.ds(pl.multiple_of(s * seg, seg), seg)
            for j in range(n_col):
                cols = slice(j * LANES, (j + 1) * LANES)
                hc_s[:M, cols] = acc[j][:M]
                hx[rows, cols] = x_s[rows, cols].astype(F32) + mod_s[2, 0:1, cols] * acc[j][M:]
            return carry

        lax.fori_loop(0, n_seg, step, 0)
        mix_in(n_seg - 1)

    pl.run_scoped(
        attention,
        pltpu.VMEM((3 * H, D // 2, Dh), U32),
        pltpu.VMEM((n_col, H * Dh, LANES), BF16),
        pltpu.VMEM((n_col, D, LANES), BF16),
        pltpu.VMEM((3 * H, ring, Dh), F32),
        pltpu.VMEM((3, D, HEAD_TILE, Dh), BF16),
        pltpu.VMEM((4, D, D + LANES), BF16),
        pltpu.VMEM((seg, D), F32),
        *[pltpu.VMEM((L, H * Dh // N_PART), F32)] * N_PART,
    )

    def mixer(out_s):
        n_chunk = S // ROWS
        rs = ROWS // N_SPLIT
        cq = D // 4
        for cp in b_copies:
            cp.wait()

        def out_copy(i, b):
            return pltpu.make_async_copy(
                out_s.at[b], out_hbm.at[pl.ds(pl.multiple_of(i * ROWS, ROWS), ROWS), :],
                sem_out.at[b])

        def mlp(i, carry):
            b = i % 2

            @pl.when(i >= 2)
            def _():
                out_copy(i - 2, b).wait()

            x1 = []
            for a in range(N_SPLIT):
                start = pl.multiple_of(i * ROWS + a * rs, rs)
                parts = []
                for g, off in enumerate((-1, 1, -2, 2)):
                    ug = u_s[pl.ds(start, rs + 2 * PAD), g * cq:(g + 1) * cq]
                    parts.append(ug[PAD + off:PAD + off + rs])
                x1.append(cond(hx[pl.ds(start, rs), :])
                          + _mm(jnp.concatenate(parts, axis=1), w2_s[...]))
            t = [_gelu(_mm(_layernorm(v), w3_s[...])) for v in x1]
            for a in range(N_SPLIT):
                start = pl.multiple_of(i * ROWS + a * rs, rs)
                y = x1[a] + _mm(t[a], w4_s[...])
                out_s[b, a * rs:(a + 1) * rs, :] = (
                    hx[pl.ds(start, rs), :] + mod(5) * y).astype(out_s.dtype)
            out_copy(i, b).start()
            return carry

        lax.fori_loop(0, n_chunk, mlp, 0)
        out_copy(n_chunk - 2, (n_chunk - 2) % 2).wait()
        out_copy(n_chunk - 1, (n_chunk - 1) % 2).wait()

    pl.run_scoped(mixer, pltpu.VMEM((2, ROWS, D), out_hbm.dtype))


@functools.partial(jax.jit, static_argnames=("A_seg_len",))
def pallas_adaLN_cond__memory_aug_recurrent_mem_tr__mixer_s_mlp__prompt_kernel(
    A_x, A_mem0, A_Wq, A_Wk, A_Wv, A_Wo, A_seg_len,
    B_x, B_w1, B_w2, B_w3, B_w4, c, w_mod,
):
    del B_x
    B, S, D = A_x.shape
    _, H, Dh = A_Wq.shape
    M = A_mem0.shape[1]
    F = B_w3.shape[1]
    assert B == 1 and Dh == LANES and M == SUB and S % ROWS == 0

    hbm = pl.BlockSpec(memory_space=pl.ANY)
    vmem = pl.BlockSpec(memory_space=pltpu.VMEM)
    dma = pltpu.SemaphoreType.DMA

    out = pl.pallas_call(
        functools.partial(_kernel, seg=int(A_seg_len)),
        out_shape=jax.ShapeDtypeStruct((S, D), A_x.dtype),
        in_specs=[hbm, vmem, hbm, hbm, hbm, hbm, hbm, hbm, hbm, hbm, vmem, hbm],
        out_specs=hbm,
        scratch_shapes=[
            pltpu.VMEM((S, D), A_x.dtype),
            pltpu.VMEM((S, D), F32),
            pltpu.VMEM((S + 2 * SUB, D), F32),
            pltpu.VMEM((6, SUB, D), F32),
            pltpu.VMEM((D, D), BF16),
            pltpu.VMEM((D, F), BF16),
            pltpu.VMEM((F, D), BF16),
            dma((2,)), dma((3,)), dma((D // LANES,)), dma((D // LANES,)),
            dma((4,)), dma((3,)), dma((2,)),
        ],
        compiler_params=pltpu.CompilerParams(vmem_limit_bytes=124 * 1024 * 1024),
    )(
        A_x.reshape(S, D), A_mem0.reshape(M, D), A_Wq, A_Wk, A_Wv,
        A_Wo.reshape(H * Dh, D), B_w1, B_w2, B_w3, B_w4, c, w_mod,
    )
    return out.reshape(B, S, D)
```
